```python
import jax
import jax.numpy as jnp

def _softmax(x, axis=-1):
    return jax.nn.softmax(x, axis=axis)

def _gelu(x):
    return jax.nn.gelu(x, approximate=True)

def _silu(x):
    return jax.nn.silu(x)

def _sigmoid(x):
    return jax.nn.sigmoid(x)

def _layernorm(x, axis=-1, eps=1e-05):
    m = jnp.mean(x, axis=axis, keepdims=True)
    v = jnp.var(x, axis=axis, keepdims=True)
    return (x - m) / jnp.sqrt(v + eps)

def _scatter_add(tgt, idx, src, axis=0):
    return tgt.at[idx].add(src)

def _segment_sum(src, seg, n):
    return jax.ops.segment_sum(src, seg, n)

class _Rng:

    def __init__(self, key):
        self._k = key

    def _next(self):
        self._k, sub = jax.random.split(self._k)
        return sub

    def normal(self, shape):
        return jax.random.normal(self._next(), shape, dtype=jnp.bfloat16)

    def randint(self, lo, hi, shape):
        return jax.random.randint(self._next(), shape, lo, hi, dtype=jnp.int32)

    def uniform(self, shape, lo=0.0, hi=1.0):
        return jax.random.uniform(self._next(), shape, jnp.bfloat16, lo, hi)

    def permutation(self, n):
        return jax.random.permutation(self._next(), n)
kernel_name = 'adaLN_cond__mha_block_cached__moe_arch_mod__prompt'

def setup_inputs():
    _rng = _Rng(jax.random.key(int.from_bytes(__import__("os").urandom(4), "little")))
    _w = lambda a: (lambda t: t.astype(jnp.bfloat16) if jnp.issubdtype(t.dtype, jnp.floating) else t)(jnp.asarray(a))

    def _A_setup():
        B, Sq, D = (1, 2048, 1024)
        H, Sk, Dh = (32, 2048, 128)
        return {'x': _w((lambda *s: _rng.normal(s) * 0.05)(B, Sq, D)), 'k_cache': _w((lambda *s: _rng.normal(s) * 0.05)(B, H, Sk, Dh)), 'v_cache': _w((lambda *s: _rng.normal(s) * 0.05)(B, H, Sk, Dh)), 'wq': _w((lambda *s: _rng.normal(s) * 0.05)(D, H * Dh) * D ** (-0.5)), 'wo': _w((lambda *s: _rng.normal(s) * 0.05)(H * Dh, D) * (H * Dh) ** (-0.5))}
    _A_in = _A_setup()

    def _B_setup():
        B, S, D, F, C = (1, 2048, 1024, 3584, 2)
        return {'x': _w((lambda *s: _rng.normal(s) * 0.05)(B, S, D)), 'w_r': _w((lambda *s: _rng.normal(s) * 0.05)(D)), 'w_gate': _w((lambda *s: _rng.normal(s) * 0.05)(D, F)), 'w_up': _w((lambda *s: _rng.normal(s) * 0.05)(D, F)), 'w_down': _w((lambda *s: _rng.normal(s) * 0.05)(F, D))}
    _B_in = _B_setup()
    return {'A_x': _A_in['x'], 'A_k_cache': _A_in['k_cache'], 'A_v_cache': _A_in['v_cache'], 'A_wq': _A_in['wq'], 'A_wo': _A_in['wo'], 'B_x': _B_in['x'], 'B_w_r': _B_in['w_r'], 'B_w_gate': _B_in['w_gate'], 'B_w_up': _B_in['w_up'], 'B_w_down': _B_in['w_down'], 'c': _w((lambda *s: _rng.normal(s) * 0.05)(1, 1024)), 'w_mod': _w((lambda *s: _rng.normal(s) * 0.05)(1024, 6 * 1024) * 1024 ** (-0.5))}

def reference(A_x, A_k_cache, A_v_cache, A_wq, A_wo, B_x, B_w_r, B_w_gate, B_w_up, B_w_down, c, w_mod):

    def _A_ref(x, k_cache, v_cache, wq, wo):
        B, Sq, D = x.shape
        H, Dh = (32, 128)
        q = (lambda x, *d: x.transpose(*d))((x @ wq).reshape(B, Sq, H, Dh), 0, 2, 1, 3)
        scores = jnp.einsum('bhqd,bhkd->bhqk', q, k_cache) * Dh ** (-0.5)
        p = _softmax(scores, axis=-1)
        o = jnp.einsum('bhqk,bhkd->bhqd', p, v_cache)
        return (lambda x, *d: x.transpose(*d))(o, 0, 2, 1, 3).reshape(B, Sq, H * Dh) @ wo

    def _B_ref(x, w_r, w_gate, w_up, w_down):
        B, S, D = x.shape
        C = 2
        r = x @ w_r
        idx = jnp.argsort(-r, axis=-1)[:, :C]
        idx_e = jnp.repeat(idx.reshape(B, C, 1), D, axis=2)
        x_sel = jnp.take_along_axis(x, idx_e, axis=1)
        g = _silu(x_sel @ w_gate)
        u = x_sel @ w_up
        y = g * u @ w_down
        r_sel = _sigmoid(jnp.take_along_axis(r, idx, axis=1))
        y = y * r_sel.reshape(B, C, 1)
        b_off = (jnp.arange(B) * S).reshape(B, 1)
        flat_idx = (idx + b_off).reshape(B * C)
        zero = (x * 0.0).reshape(B * S, D)
        upd = _scatter_add(zero, flat_idx, y.reshape(B * C, D), axis=0)
        return x + upd.reshape(B, S, D)
    x = A_x
    mod = (_silu(c) @ w_mod).reshape(c.shape[0], 6, 1, -1)
    sa, ca, ga, sb, cb, gb = (mod[:, 0].copy(), mod[:, 1].copy(), mod[:, 2].copy(), mod[:, 3].copy(), mod[:, 4].copy(), mod[:, 5].copy())
    h = _layernorm(x, axis=-1) * (1 + ca) + sa
    x = x + ga * _A_ref(h, A_k_cache, A_v_cache, A_wq, A_wo)
    h = _layernorm(x, axis=-1) * (1 + cb) + sb
    x = x + gb * _B_ref(h, B_w_r, B_w_gate, B_w_up, B_w_down)
    return x
```

```python
import functools

import jax
import jax.numpy as jnp
import jax.experimental.pallas as pl
import jax.experimental.pallas.tpu as pltpu

S = 2048
D = 1024
H = 32
DH = 128
F = 3584
R = 256
NR = S // R
NSLOT = 4
KD = D // 128
FB = F // 128
EPS = 1e-5
LOG2E = 1.4426950408889634
QSCALE = (DH ** -0.5) * LOG2E
BF = jnp.bfloat16
F32 = jnp.float32


def _kernel(x_hbm, k_hbm, v_hbm, wq_hbm, wo_hbm, wr_hbm, wg_hbm, wu_hbm, wd_hbm,
            c_hbm, wm_hbm, out_hbm,
            x_buf, o_stage, h_buf, acc, q_buf, o_buf, k_buf, v_buf, wq_buf, wo_buf, wm_buf,
            wm1_buf, wg_buf, wu_buf, wd_buf, c_buf, wr_buf, scol, mod_buf, r_buf,
            sem_pk, sem_x, sem_m1, sem_small, sem_moe, sem_out, sem_fix):

    def packet(h, slot):
        return [
            pltpu.make_async_copy(k_hbm.at[h], k_buf.at[slot], sem_pk.at[slot, 0]),
            pltpu.make_async_copy(wq_hbm.at[:, pl.ds(h * DH, DH)], wq_buf.at[slot], sem_pk.at[slot, 1]),
            pltpu.make_async_copy(v_hbm.at[h], v_buf.at[slot], sem_pk.at[slot, 2]),
            pltpu.make_async_copy(wo_hbm.at[pl.ds(h * DH, DH), :], wo_buf.at[slot], sem_pk.at[slot, 3]),
            pltpu.make_async_copy(wm_hbm.at[:, pl.ds(2 * D + h * 128, 128)], wm_buf.at[slot], sem_pk.at[slot, 4]),
        ]

    def x_copy(r0, n, i):
        return pltpu.make_async_copy(x_hbm.at[pl.ds(r0, n), :], x_buf.at[pl.ds(r0, n), :], sem_x.at[i])

    M1C = 4
    MR = D // M1C

    def m1_copy(i):
        return pltpu.make_async_copy(wm_hbm.at[pl.ds(i * MR, MR), pl.ds(0, 2 * D)],
                                     wm1_buf.at[pl.ds(i * MR, MR), :], sem_m1.at[i])

    def moe_copies(j):
        return [
            pltpu.make_async_copy(wg_hbm.at[:, pl.ds(j * 128, 128)], wg_buf.at[j], sem_moe.at[0]),
            pltpu.make_async_copy(wu_hbm.at[:, pl.ds(j * 128, 128)], wu_buf.at[j], sem_moe.at[1]),
            pltpu.make_async_copy(wd_hbm.at[pl.ds(j * 128, 128), :], wd_buf.at[j], sem_moe.at[2]),
        ]

    def out_copy(r):
        return pltpu.make_async_copy(o_stage.at[pl.ds(r * R, R), :], out_hbm.at[pl.ds(r * R, R), :], sem_out.at[r])

    c_copy = pltpu.make_async_copy(c_hbm, c_buf, sem_small.at[0])
    wr_copy = pltpu.make_async_copy(wr_hbm, wr_buf, sem_small.at[1])

    X0 = 3 * R
    c_copy.start()
    for i in range(M1C):
        m1_copy(i).start()
    x_copy(0, X0, 0).start()
    pk0 = packet(0, 0)
    for cp in pk0:
        cp.start()
    x_copy(X0, S - X0, 1).start()
    for cp in packet(1, 1):
        cp.start()
    wr_copy.start()

    c_copy.wait()
    cf = c_buf[...].astype(F32)
    sc = (cf * jax.nn.sigmoid(cf)).astype(BF)
    sc16 = jnp.broadcast_to(sc, (16, D))
    scf = sc.astype(F32)
    for j in range(KD):
        blk = jnp.broadcast_to(scf[:, j * 128:(j + 1) * 128], (128, 128))
        scol[j * 128:(j + 1) * 128, :] = blk.T
    m1 = jnp.zeros((16, 2 * D), F32)
    for i in range(M1C):
        m1_copy(i).wait()
        m1 = m1 + jnp.dot(sc16[:, i * MR:(i + 1) * MR], wm1_buf[i * MR:(i + 1) * MR, :],
                          preferred_element_type=F32)
    m1 = m1[0:1, :].astype(BF).astype(F32)
    sa = m1[:, 0:D]
    ca1 = (1.0 + m1[:, D:2 * D]).astype(BF).astype(F32)

    def ln_mod(xf, mul, add):
        mu = jnp.mean(xf, axis=-1, keepdims=True)
        d = xf - mu
        var = jnp.mean(d * d, axis=-1, keepdims=True)
        return d * jax.lax.rsqrt(var + EPS) * mul + add

    def stage_ln(r):
        rows = pl.ds(r * R, R)
        hh = ln_mod(x_buf[rows, :].astype(F32), ca1, sa).astype(BF)
        for j in range(KD):
            h_buf[j, rows, :] = hh[:, j * 128:(j + 1) * 128]

    def stage_q(r, slot):
        rows = pl.ds(r * R, R)
        wq = wq_buf.at[slot]
        q = None
        for j in range(KD):
            t = jnp.dot(h_buf[j, rows, :], wq[j * 128:(j + 1) * 128, :], preferred_element_type=F32)
            q = t if q is None else q + t
        q_buf[rows, :] = (q * QSCALE).astype(BF)

    def stage_s(r, slot):
        rows = pl.ds(r * R, R)
        return jax.lax.dot_general(q_buf[rows, :], k_buf[slot], (((1,), (1,)), ((), ())),
                                   preferred_element_type=F32)

    def stage_pv(s, slot):
        m = jnp.max(s, axis=-1, keepdims=True)
        p = jnp.exp2(s - m)
        l = jnp.sum(p, axis=-1, keepdims=True)
        o = jnp.dot(p.astype(BF), v_buf[slot], preferred_element_type=F32)
        return (o / l).astype(BF)

    def stage_o(o, r, slot, mode):
        rows = pl.ds(r * R, R)
        t = jnp.dot(o, wo_buf[slot], preferred_element_type=F32)
        if mode == "first":
            acc[rows, :] = t
        elif mode == "mid":
            acc[rows, :] = acc[rows, :] + t
        else:
            ga, cb1, sb, gb, wr = fin_consts
            x1 = (x_buf[rows, :].astype(F32) + ga * (acc[rows, :] + t)).astype(BF)
            x_buf[rows, :] = x1
            xf = x1.astype(F32)
            h2 = ln_mod(xf, cb1, sb).astype(BF).astype(F32)
            r_buf[rows, :] = jnp.sum(h2 * wr, axis=-1, keepdims=True)
            o_stage[rows, :] = (xf + gb * h2).astype(BF)
            out_copy(r).start()

    def stage_mod(h, slot):
        w = wm_buf[slot].astype(F32) * scol[...]
        mod_buf[h] = jnp.broadcast_to(jnp.sum(w, axis=0, keepdims=True), (8, 128))

    def mod_row(i):
        return jnp.concatenate([mod_buf[i * KD + j][0:1, :] for j in range(KD)], axis=1).astype(BF).astype(F32)

    def body(h, first, last):
        slot = h % NSLOT
        pslot = (h - 1) % NSLOT
        nslot = (h + 1) % NSLOT
        stage_mod(h, slot)
        if last:
            fin_consts.extend([mod_row(0), (1.0 + mod_row(2)).astype(BF).astype(F32), mod_row(1), mod_row(3),
                               wr_buf[...].astype(F32).reshape(1, D)])
        o_prev = None
        for r in range(NR):
            if first and r + 3 < NR:
                if r == 0:
                    x_copy(X0, S - X0, 1).wait()
                stage_ln(r + 3)
            s = stage_s(r, slot)
            if r == 0:
                if not first:
                    stage_o(o_buf[...], NR - 1, pslot, "mid")
            else:
                stage_o(o_prev, r - 1, slot, "first" if first else ("last" if last else "mid"))
            if r + 2 < NR:
                stage_q(r + 2, slot)
            elif not last:
                stage_q(r + 2 - NR, nslot)
            o_prev = stage_pv(s, slot)
        o_buf[...] = o_prev

    fin_consts = []

    x_copy(0, X0, 0).wait()
    for r in range(3):
        stage_ln(r)
    pk0[1].wait()
    stage_q(0, 0)
    stage_q(1, 0)
    pk0[0].wait()
    pk0[2].wait()
    pk0[3].wait()
    pk0[4].wait()
    for cp in packet(1, 1):
        cp.wait()
    for cp in packet(2, 2):
        cp.start()
    acc[pl.ds(S - R, R), :] = jnp.zeros((R, D), F32)
    body(0, True, False)

    def loop(h, carry):
        @pl.when(h + 2 < H)
        def _():
            for cp in packet(h + 2, (h + 2) % NSLOT):
                cp.start()

        @pl.when(h <= FB)
        def _():
            for cp in moe_copies(h - 1):
                cp.start()

        for cp in packet(h + 1, (h + 1) % NSLOT):
            cp.wait()
        body(h, False, False)
        return carry

    jax.lax.fori_loop(1, H - 1, loop, 0)

    wr_copy.wait()
    body(H - 1, False, True)
    stage_o(o_buf[...], NR - 1, (H - 1) % NSLOT, "last")
    ga, cb1, sb, gb, wr = fin_consts

    rr = r_buf[...]
    row = jax.lax.broadcasted_iota(jnp.int32, (S, 1), 0)
    m1v = jnp.max(rr)
    i1 = jnp.clip(jnp.min(jnp.where(rr == m1v, row, S)), 0, S - 1)
    rr2 = jnp.where(row == i1, -jnp.inf, rr)
    m2v = jnp.max(rr2)
    i2 = jnp.clip(jnp.min(jnp.where(rr2 == m2v, row, S)), 0, S - 1)

    b1 = pl.multiple_of((i1 // 16) * 16, 16)
    b2 = pl.multiple_of((i2 // 16) * 16, 16)
    xs = jnp.concatenate([x_buf[pl.ds(b1, 16), :], x_buf[pl.ds(b2, 16), :]], axis=0).astype(F32)
    h2 = ln_mod(xs, cb1, sb).astype(BF)
    h2f = h2.astype(F32)

    for t in range(3):
        pltpu.make_async_copy(wg_buf if t == 0 else (wu_buf if t == 1 else wd_buf),
                              wg_buf if t == 0 else (wu_buf if t == 1 else wd_buf), sem_moe.at[t]).wait()
    y = jnp.zeros((32, D), F32)
    for j in range(FB):
        g = jnp.dot(h2, wg_buf[j], preferred_element_type=F32)
        u = jnp.dot(h2, wu_buf[j], preferred_element_type=F32)
        a = (g * jax.nn.sigmoid(g) * u).astype(BF)
        y = y + jnp.dot(a, wd_buf[j], preferred_element_type=F32)

    g1 = jax.nn.sigmoid(jnp.full((1, 1), m1v, F32))
    g2 = jax.nn.sigmoid(jnp.full((1, 1), m2v, F32))
    row16 = jax.lax.broadcasted_iota(jnp.int32, (16, D), 0)

    for r in range(NR):
        out_copy(r).wait()

    ya = y[0:16] * g1
    yb = y[16:32] * g2
    u1 = jnp.where(row16 == i1 - b1, ya, jnp.where(row16 == i2 - b1, yb, 0.0))
    u2 = jnp.where(row16 == i2 - b2, yb, jnp.where(row16 == i1 - b2, ya, 0.0))
    o_stage[pl.ds(b1, 16), :] = (xs[0:16] + gb * (h2f[0:16] + u1)).astype(BF)
    o_stage[pl.ds(b2, 16), :] = (xs[16:32] + gb * (h2f[16:32] + u2)).astype(BF)

    f1 = pltpu.make_async_copy(o_stage.at[pl.ds(b1, 16), :], out_hbm.at[pl.ds(b1, 16), :], sem_fix.at[0])
    f2 = pltpu.make_async_copy(o_stage.at[pl.ds(b2, 16), :], out_hbm.at[pl.ds(b2, 16), :], sem_fix.at[1])
    f1.start()

    @pl.when(b1 != b2)
    def _():
        f2.start()
        f2.wait()

    f1.wait()


@jax.jit
def pallas_adaLN_cond__mha_block_cached__moe_arch_mod__prompt_kernel(
    A_x: jax.Array,
    A_k_cache: jax.Array,
    A_v_cache: jax.Array,
    A_wq: jax.Array,
    A_wo: jax.Array,
    B_x: jax.Array,
    B_w_r: jax.Array,
    B_w_gate: jax.Array,
    B_w_up: jax.Array,
    B_w_down: jax.Array,
    c: jax.Array,
    w_mod: jax.Array,
):
    any_spec = pl.BlockSpec(memory_space=pl.ANY)
    out = pl.pallas_call(
        _kernel,
        out_shape=jax.ShapeDtypeStruct((S, D), BF),
        in_specs=[any_spec] * 11,
        out_specs=any_spec,
        scratch_shapes=[
            pltpu.VMEM((S, D), BF),
            pltpu.VMEM((S, D), BF),
            pltpu.VMEM((KD, S, 128), BF),
            pltpu.VMEM((S, D), F32),
            pltpu.VMEM((S, DH), BF),
            pltpu.VMEM((R, DH), BF),
            pltpu.VMEM((NSLOT, S, DH), BF),
            pltpu.VMEM((NSLOT, S, DH), BF),
            pltpu.VMEM((NSLOT, D, DH), BF),
            pltpu.VMEM((NSLOT, DH, D), BF),
            pltpu.VMEM((NSLOT, D, 128), BF),
            pltpu.VMEM((D, 2 * D), BF),
            pltpu.VMEM((FB, D, 128), BF),
            pltpu.VMEM((FB, D, 128), BF),
            pltpu.VMEM((FB, 128, D), BF),
            pltpu.VMEM((1, D), BF),
            pltpu.VMEM((D,), BF),
            pltpu.VMEM((D, 128), F32),
            pltpu.VMEM((H, 8, 128), F32),
            pltpu.VMEM((S, 1), F32),
            pltpu.SemaphoreType.DMA((NSLOT, 5)),
            pltpu.SemaphoreType.DMA((2,)),
            pltpu.SemaphoreType.DMA((4,)),
            pltpu.SemaphoreType.DMA((2,)),
            pltpu.SemaphoreType.DMA((3,)),
            pltpu.SemaphoreType.DMA((NR,)),
            pltpu.SemaphoreType.DMA((2,)),
        ],
        compiler_params=pltpu.CompilerParams(vmem_limit_bytes=110 << 20),
    )(
        A_x.reshape(S, D),
        A_k_cache.reshape(H, S, DH),
        A_v_cache.reshape(H, S, DH),
        A_wq,
        A_wo,
        B_w_r,
        B_w_gate,
        B_w_up,
        B_w_down,
        c,
        w_mod,
    )
    return out.reshape(1, S, D)
```

```python
import jax
import jax.numpy as jnp
import jax.experimental.pallas as pl
import jax.experimental.pallas.tpu as pltpu

S = 2048
D = 1024
H = 32
DH = 128
F = 3584
KB = 512
NKB = S // KB
RX = 512
NX = S // RX
RC = 512
NC = S // RC
KD = D // 128
FB = F // 128
M1C = 4
MR = D // M1C
EPS = 1e-5
LOG2E = 1.4426950408889634
QSCALE = (DH ** -0.5) * LOG2E
BF = jnp.bfloat16
F32 = jnp.float32


def _ln_mod(xf, mul, add):
    mu = jnp.mean(xf, axis=-1, keepdims=True)
    d = xf - mu
    var = jnp.mean(d * d, axis=-1, keepdims=True)
    return d * jax.lax.rsqrt(var + EPS) * mul + add


def _mm(a, b):
    return jnp.dot(a, b, preferred_element_type=F32)


def _kernel(x_hbm, k_hbm, v_hbm, wq_hbm, wo_hbm, wr_hbm, wg_hbm, wu_hbm, wd_hbm,
            c_hbm, wm_hbm, out_hbm,
            x_buf, o_stage, h_buf, acc, s_buf, m_buf, of_buf, l_buf,
            q_buf, k_buf, v_buf, wq_buf, wo_buf, wm_buf, wq0_buf,
            wm1_buf, wg_buf, wu_buf, wd_buf, c_buf, wr_buf, scol, mod_buf, fin_buf, r_buf,
            sem_pk, sem_x, sem_m1, sem_small, sem_moe, sem_out, sem_fix):
    def cp_k(h, slot):
        return pltpu.make_async_copy(k_hbm.at[h], k_buf.at[slot], sem_pk.at[slot, 0])

    def cp_v(h, slot):
        return pltpu.make_async_copy(v_hbm.at[h], v_buf.at[slot], sem_pk.at[slot, 1])

    def cp_wq(h, slot):
        return pltpu.make_async_copy(wq_hbm.at[:, pl.ds(h * DH, DH)], wq_buf.at[slot], sem_pk.at[slot, 2])

    def cp_wo(h, slot):
        return pltpu.make_async_copy(wo_hbm.at[pl.ds(h * DH, DH), :], wo_buf.at[slot], sem_pk.at[slot, 3])

    def cp_wm(h, slot):
        return pltpu.make_async_copy(wm_hbm.at[:, pl.ds(2 * D + h * 128, 128)], wm_buf.at[slot], sem_pk.at[slot, 4])

    def packet(h, slot, last=False):
        cps = [] if last else [cp_wq(h + 1, slot)]
        cps += [cp_v(h, slot), cp_wm(h, slot)]
        if not last:
            cps.append(cp_k(h + 1, slot))
        cps.append(cp_wo(h, slot))
        return cps

    def x_copy(i):
        return pltpu.make_async_copy(x_hbm.at[pl.ds(i * RX, RX), :], x_buf.at[pl.ds(i * RX, RX), :], sem_x.at[i])

    def m1_copy(i):
        return pltpu.make_async_copy(wm_hbm.at[pl.ds(i * MR, MR), pl.ds(0, 2 * D)],
                                     wm1_buf.at[pl.ds(i * MR, MR), :], sem_m1.at[i])

    def moe_copies(j):
        return [
            pltpu.make_async_copy(wg_hbm.at[:, pl.ds(j * 128, 128)], wg_buf.at[j], sem_moe.at[0]),
            pltpu.make_async_copy(wu_hbm.at[:, pl.ds(j * 128, 128)], wu_buf.at[j], sem_moe.at[1]),
            pltpu.make_async_copy(wd_hbm.at[pl.ds(j * 128, 128), :], wd_buf.at[j], sem_moe.at[2]),
        ]

    def out_copy(r0, i):
        return pltpu.make_async_copy(o_stage.at[pl.ds(r0, RC), :], out_hbm.at[pl.ds(r0, RC), :], sem_out.at[i])

    c_copy = pltpu.make_async_copy(c_hbm, c_buf, sem_small.at[0])
    wr_copy = pltpu.make_async_copy(wr_hbm, wr_buf, sem_small.at[1])
    wq0_copy = pltpu.make_async_copy(wq_hbm.at[:, pl.ds(0, DH)], wq0_buf, sem_small.at[2])

    def stage_q(rows, wq):
        q = None
        for j in range(KD):
            t = _mm(h_buf[j, rows, :], wq[j * 128:(j + 1) * 128, :])
            q = t if q is None else q + t
        return (q * QSCALE).astype(BF)

    def qk_round(q, t, k_ref, sbuf, mx):
        s = jax.lax.dot_general(q, k_ref[t * KB:(t + 1) * KB, :], (((1,), (1,)), ((), ())),
                                preferred_element_type=F32)
        sbuf[:, t * KB:(t + 1) * KB] = s
        for j in range(KB // 128):
            sj = s[:, j * 128:(j + 1) * 128]
            mx = sj if mx is None else jnp.maximum(mx, sj)
        return mx

    def row_max(mx):
        return jnp.broadcast_to(jnp.max(mx, axis=-1, keepdims=True), mx.shape)

    def stage_s(k_ref):
        mx = None
        for t in range(NKB):
            mx = qk_round(q_buf[...], t, k_ref, s_buf, mx)
        m_buf[...] = row_max(mx)

    def stage_pv(rows, v_ref):
        m = m_buf[rows, :]
        m = jnp.concatenate([m] * (KB // 128), axis=1)
        o = None
        for t in range(NKB):
            p = jnp.exp2(s_buf[rows, t * KB:(t + 1) * KB] - m)
            l = p[:, 0:128]
            for j in range(1, KB // 128):
                l = l + p[:, j * 128:(j + 1) * 128]
            l_buf[t, rows, :] = l
            ot = _mm(p.astype(BF), v_ref[t * KB:(t + 1) * KB, :])
            o = ot if o is None else o + ot
        return o

    def normalize(o, rows):
        l = l_buf[0, rows, :]
        for t in range(1, NKB):
            l = l + l_buf[t, rows, :]
        l = jnp.sum(l, axis=-1, keepdims=True)
        return (o * pltpu.reciprocal(l, full_range=False)).astype(BF)

    def stage_mod(h, slot):
        w = wm_buf[slot].astype(F32) * scol[...]
        mod_buf[h] = jnp.broadcast_to(jnp.sum(w, axis=0, keepdims=True), (8, 128))

    def head_step(h, slot):
        allr = slice(None)
        stage_mod(h, slot)
        q_buf[...] = stage_q(allr, wq_buf.at[slot])
        o = stage_pv(allr, v_buf.at[slot])
        stage_s(k_buf.at[slot])
        acc[...] = acc[...] + _mm(normalize(o, allr), wo_buf[slot])

    c_copy.start()
    for i in range(M1C):
        m1_copy(i).start()

    c_copy.wait()
    cf = c_buf[...].astype(F32)
    sc = (cf * jax.nn.sigmoid(cf)).astype(BF)
    sc16 = jnp.broadcast_to(sc, (16, D))
    scf = sc.astype(F32)
    for j in range(KD):
        blk = jnp.broadcast_to(scf[:, j * 128:(j + 1) * 128], (128, 128))
        scol[j * 128:(j + 1) * 128, :] = blk.T
    m1 = jnp.zeros((16, 2 * D), F32)
    for i in range(M1C):
        m1_copy(i).wait()
        if i == M1C - 2:
            wq0_copy.start()
            x_copy(0).start()
        m1 = m1 + _mm(sc16[:, i * MR:(i + 1) * MR], wm1_buf[i * MR:(i + 1) * MR, :])
    m1 = m1[0:1, :].astype(BF).astype(F32)
    sa = m1[:, 0:D]
    ca1 = (1.0 + m1[:, D:2 * D]).astype(BF).astype(F32)

    acc[...] = jnp.zeros((S, D), F32)
    wq0_copy.wait()
    for i in range(NX):
        rows = pl.ds(i * RX, RX)
        if i + 1 < NX:
            x_copy(i + 1).start()
        else:
            cp_k(0, 1).start()
        x_copy(i).wait()
        hh = _ln_mod(x_buf[rows, :].astype(F32), ca1, sa).astype(BF)
        for j in range(KD):
            h_buf[j, rows, :] = hh[:, j * 128:(j + 1) * 128]
        q_buf[rows, :] = stage_q(rows, wq0_buf)
    for cp in packet(0, 0):
        cp.start()
    wr_copy.start()
    cp_k(0, 1).wait()
    stage_s(k_buf.at[1])

    def loop(h, carry):
        slot = h % 2

        @pl.when(h < FB)
        def _():
            for cp in moe_copies(h):
                cp.start()

        @pl.when(h + 2 < H)
        def _():
            cp_wq(h + 2, 1 - slot).start()
            cp_k(h + 2, 1 - slot).start()

        cp_v(h + 1, 1 - slot).start()
        cp_wm(h + 1, 1 - slot).start()
        cp_wo(h + 1, 1 - slot).start()
        for cp in packet(h, slot):
            cp.wait()
        head_step(h, slot)
        return carry

    jax.lax.fori_loop(0, H - 1, loop, 0)

    for cp in packet(H - 1, 1, last=True):
        cp.wait()
    wr_copy.wait()
    stage_mod(H - 1, 1)

    def mod_row(i):
        return jnp.concatenate([mod_buf[i * KD + j][0:1, :] for j in range(KD)], axis=1).astype(BF).astype(F32)

    cb1 = (1.0 + mod_row(2)).astype(BF).astype(F32)
    sb, gb = mod_row(1), mod_row(3)
    wr = wr_buf[...].astype(F32).reshape(1, D)
    for i, row in enumerate([mod_row(0), cb1 * wr, gb * cb1, gb * sb]):
        fin_buf[i] = jnp.broadcast_to(row, (8, D))
    r_const = jnp.sum(sb * wr, axis=-1, keepdims=True)

    def fin(i):
        return fin_buf[i][0:1, :]

    def last_pv(r0):
        rows = pl.ds(r0, RC)
        of_buf[rows, :] = stage_pv(rows, v_buf.at[1])

    def last_out(r0, i):
        rows = pl.ds(r0, RC)
        att = acc[rows, :] + _mm(normalize(of_buf[rows, :], rows), wo_buf[1])
        x1 = x_buf[rows, :].astype(F32) + fin(0) * att
        acc[rows, :] = x1
        mu = jnp.mean(x1, axis=-1, keepdims=True)
        d = x1 - mu
        rstd = jax.lax.rsqrt(jnp.mean(d * d, axis=-1, keepdims=True) + EPS)
        r_buf[rows, :] = jnp.sum(d * fin(1), axis=-1, keepdims=True) * rstd
        o_stage[rows, :] = ((x1 + fin(3)) + (d * rstd) * fin(2)).astype(BF)
        out_copy(r0, i).start()

    last_pv(0)

    def last_loop(i, carry):
        last_out(pl.multiple_of((i - 1) * RC, RC), i - 1)
        last_pv(pl.multiple_of(i * RC, RC))
        return carry

    jax.lax.fori_loop(1, NC, last_loop, 0)
    last_out((NC - 1) * RC, NC - 1)

    rr = r_buf[...] + r_const
    row = jax.lax.broadcasted_iota(jnp.int32, (S, 1), 0)
    m1v = jnp.max(rr)
    i1 = jnp.clip(jnp.min(jnp.where(rr == m1v, row, S)), 0, S - 1)
    rr2 = jnp.where(row == i1, -jnp.inf, rr)
    m2v = jnp.max(rr2)
    i2 = jnp.clip(jnp.min(jnp.where(rr2 == m2v, row, S)), 0, S - 1)

    b1 = pl.multiple_of((i1 // 16) * 16, 16)
    b2 = pl.multiple_of((i2 // 16) * 16, 16)
    xs = jnp.concatenate([acc[pl.ds(b1, 16), :], acc[pl.ds(b2, 16), :]], axis=0)
    h2 = _ln_mod(xs, cb1, sb).astype(BF)
    h2f = h2.astype(F32)

    for t, buf in enumerate((wg_buf, wu_buf, wd_buf)):
        pltpu.make_async_copy(buf, buf, sem_moe.at[t]).wait()
    y = jnp.zeros((32, D), F32)
    for j in range(FB):
        g = _mm(h2, wg_buf[j])
        u = _mm(h2, wu_buf[j])
        a = (g * jax.nn.sigmoid(g) * u).astype(BF)
        y = y + _mm(a, wd_buf[j])

    g1 = jax.nn.sigmoid(jnp.full((1, 1), m1v, F32))
    g2 = jax.nn.sigmoid(jnp.full((1, 1), m2v, F32))
    row16 = jax.lax.broadcasted_iota(jnp.int32, (16, D), 0)

    for i in range(NC):
        out_copy(i * RC, i).wait()

    ya = y[0:16] * g1
    yb = y[16:32] * g2
    u1 = jnp.where(row16 == i1 - b1, ya, jnp.where(row16 == i2 - b1, yb, 0.0))
    u2 = jnp.where(row16 == i2 - b2, yb, jnp.where(row16 == i1 - b2, ya, 0.0))
    o_stage[pl.ds(b1, 16), :] = (xs[0:16] + gb * (h2f[0:16] + u1)).astype(BF)
    o_stage[pl.ds(b2, 16), :] = (xs[16:32] + gb * (h2f[16:32] + u2)).astype(BF)

    f1 = pltpu.make_async_copy(o_stage.at[pl.ds(b1, 16), :], out_hbm.at[pl.ds(b1, 16), :], sem_fix.at[0])
    f2 = pltpu.make_async_copy(o_stage.at[pl.ds(b2, 16), :], out_hbm.at[pl.ds(b2, 16), :], sem_fix.at[1])
    f1.start()

    @pl.when(b1 != b2)
    def _():
        f2.start()
        f2.wait()

    f1.wait()


@jax.jit
def pallas_adaLN_cond__mha_block_cached__moe_arch_mod__prompt_kernel(
    A_x: jax.Array,
    A_k_cache: jax.Array,
    A_v_cache: jax.Array,
    A_wq: jax.Array,
    A_wo: jax.Array,
    B_x: jax.Array,
    B_w_r: jax.Array,
    B_w_gate: jax.Array,
    B_w_up: jax.Array,
    B_w_down: jax.Array,
    c: jax.Array,
    w_mod: jax.Array,
):
    any_spec = pl.BlockSpec(memory_space=pl.ANY)
    out = pl.pallas_call(
        _kernel,
        out_shape=jax.ShapeDtypeStruct((S, D), BF),
        in_specs=[any_spec] * 11,
        out_specs=any_spec,
        scratch_shapes=[
            pltpu.VMEM((S, D), BF),
            pltpu.VMEM((S, D), BF),
            pltpu.VMEM((KD, S, 128), BF),
            pltpu.VMEM((S, D), F32),
            pltpu.VMEM((S, S), F32),
            pltpu.VMEM((S, 128), F32),
            pltpu.VMEM((S, 128), F32),
            pltpu.VMEM((NKB, S, 128), F32),
            pltpu.VMEM((S, DH), BF),
            pltpu.VMEM((2, S, DH), BF),
            pltpu.VMEM((2, S, DH), BF),
            pltpu.VMEM((2, D, DH), BF),
            pltpu.VMEM((2, DH, D), BF),
            pltpu.VMEM((2, D, 128), BF),
            pltpu.VMEM((D, DH), BF),
            pltpu.VMEM((D, 2 * D), BF),
            pltpu.VMEM((FB, D, 128), BF),
            pltpu.VMEM((FB, D, 128), BF),
            pltpu.VMEM((FB, 128, D), BF),
            pltpu.VMEM((1, D), BF),
            pltpu.VMEM((D,), BF),
            pltpu.VMEM((D, 128), F32),
            pltpu.VMEM((H, 8, 128), F32),
            pltpu.VMEM((5, 8, D), F32),
            pltpu.VMEM((S, 1), F32),
            pltpu.SemaphoreType.DMA((2, 5)),
            pltpu.SemaphoreType.DMA((NX,)),
            pltpu.SemaphoreType.DMA((M1C,)),
            pltpu.SemaphoreType.DMA((3,)),
            pltpu.SemaphoreType.DMA((3,)),
            pltpu.SemaphoreType.DMA((NC,)),
            pltpu.SemaphoreType.DMA((2,)),
        ],
        compiler_params=pltpu.CompilerParams(vmem_limit_bytes=120 << 20, disable_bounds_checks=True),
    )(
        A_x.reshape(S, D),
        A_k_cache.reshape(H, S, DH),
        A_v_cache.reshape(H, S, DH),
        A_wq,
        A_wo,
        B_w_r,
        B_w_gate,
        B_w_up,
        B_w_down,
        c,
        w_mod,
    )
    return out.reshape(1, S, D)
```

```python
import jax
import jax.numpy as jnp
import jax.experimental.pallas as pl
import jax.experimental.pallas.tpu as pltpu

S = 2048
D = 1024
H = 32
DH = 128
F = 3584
KB = 512
NKB = S // KB
RX = 512
NX = S // RX
RG = 16
RC = 512
NC = S // RC
KD = D // 128
FB = F // 128
M1C = 4
MR = D // M1C
EPS = 1e-5
LOG2E = 1.4426950408889634
QSCALE = (DH ** -0.5) * LOG2E
BF = jnp.bfloat16
F32 = jnp.float32


def _ln_mod(xf, mul, add):
    mu = jnp.mean(xf, axis=-1, keepdims=True)
    d = xf - mu
    var = jnp.mean(d * d, axis=-1, keepdims=True)
    return d * jax.lax.rsqrt(var + EPS) * mul + add


def _mm(a, b):
    return jnp.dot(a, b, preferred_element_type=F32)


def _kernel(x_hbm, k_hbm, v_hbm, wq_hbm, wo_hbm, wr_hbm, wg_hbm, wu_hbm, wd_hbm,
            c_hbm, wm_hbm, out_hbm,
            x_buf, o_stage, h_buf, acc, s_buf, m_buf, of_buf, l_buf,
            q_buf, k_buf, v_buf, wq_buf, wo_buf, wm_buf, wq0_buf,
            wm1_buf, wg_buf, wu_buf, wd_buf, c_buf, wr_buf, scol, sa_col, mod_buf, fin_buf, r_buf, flag,
            sem_pk, sem_x, sem_m1, sem_small, sem_moe, sem_out, sem_fix, sem_fence):
    def cp_k(h, slot):
        return pltpu.make_async_copy(k_hbm.at[h], k_buf.at[slot], sem_pk.at[slot, 0])

    def cp_v(h, slot):
        return pltpu.make_async_copy(v_hbm.at[h], v_buf.at[slot], sem_pk.at[slot, 1])

    def cp_wq(h, slot):
        return pltpu.make_async_copy(wq_hbm.at[:, pl.ds(h * DH, DH)], wq_buf.at[slot], sem_pk.at[slot, 2])

    def cp_wo(h, slot):
        return pltpu.make_async_copy(wo_hbm.at[pl.ds(h * DH, DH), :], wo_buf.at[slot], sem_pk.at[slot, 3])

    def cp_wm(h, slot):
        return pltpu.make_async_copy(wm_hbm.at[:, pl.ds(2 * D + h * 128, 128)], wm_buf.at[slot], sem_pk.at[slot, 4])

    def packet(h, slot, last=False):
        cps = [] if last else [cp_wq(h + 1, slot)]
        cps += [cp_v(h, slot), cp_wm(h, slot)]
        if not last:
            cps.append(cp_k(h + 1, slot))
        cps.append(cp_wo(h, slot))
        return cps

    def x_copy(i):
        rows = pl.ds(i * RX, RX)
        return pltpu.make_async_copy(x_hbm.at[rows, :], x_buf.at[rows, :], sem_x.at[i])

    def m1_copy(k, i):
        return pltpu.make_async_copy(wm_hbm.at[pl.ds(i * MR, MR), pl.ds(k * D, D)],
                                     wm1_buf.at[k, pl.ds(i * MR, MR), :], sem_m1.at[k, i])

    def moe_copies(j):
        return [
            pltpu.make_async_copy(wg_hbm.at[:, pl.ds(j * 128, 128)], wg_buf.at[j], sem_moe.at[0]),
            pltpu.make_async_copy(wu_hbm.at[:, pl.ds(j * 128, 128)], wu_buf.at[j], sem_moe.at[1]),
        ]

    def wd_copy(n):
        return pltpu.make_async_copy(wd_hbm.at[:, pl.ds(n * 128, 128)], wd_buf.at[n], sem_moe.at[2])

    def out_copy(r0, i):
        return pltpu.make_async_copy(o_stage.at[pl.ds(r0, RC), :], out_hbm.at[pl.ds(r0, RC), :], sem_out.at[i])

    c_copy = pltpu.make_async_copy(c_hbm, c_buf, sem_small.at[0])
    wr_copy = pltpu.make_async_copy(wr_hbm, wr_buf, sem_small.at[1])
    wq0_copy = pltpu.make_async_copy(wq_hbm.at[:, pl.ds(0, DH)], wq0_buf, sem_small.at[2])

    def start_in_order(*cps):
        for cp in cps:
            cp.start()
            pl.semaphore_signal(sem_fence, 1)
            pl.semaphore_wait(sem_fence, 1)

    def q_bias(wq):
        return jnp.sum(wq[...].astype(F32) * sa_col[...], axis=0, keepdims=True)

    def stage_q(wq):
        q = None
        for j in range(KD):
            t = _mm(h_buf[j], wq[j * 128:(j + 1) * 128, :])
            q = t if q is None else q + t
        return ((q + q_bias(wq)) * QSCALE).astype(BF)

    def qk_round(q, t, k_ref, sbuf, mx):
        s = jax.lax.dot_general(q, k_ref[t * KB:(t + 1) * KB, :], (((1,), (1,)), ((), ())),
                                preferred_element_type=F32)
        sbuf[:, t * KB:(t + 1) * KB] = s
        for j in range(KB // 128):
            sj = s[:, j * 128:(j + 1) * 128]
            mx = sj if mx is None else jnp.maximum(mx, sj)
        return mx

    def row_max(mx):
        return jnp.broadcast_to(jnp.max(mx, axis=-1, keepdims=True), mx.shape)

    def stage_s(q, k_ref):
        mx = None
        for t in range(NKB):
            mx = qk_round(q, t, k_ref, s_buf, mx)
        m_buf[...] = row_max(mx)

    def stage_pv(rows, v_ref):
        m = m_buf[rows, :]
        m = jnp.concatenate([m] * (KB // 128), axis=1)
        o = None
        for t in range(NKB):
            p = jnp.exp2(s_buf[rows, t * KB:(t + 1) * KB] - m)
            l = p[:, 0:128]
            for j in range(1, KB // 128):
                l = l + p[:, j * 128:(j + 1) * 128]
            l_buf[t, rows, :] = l
            ot = _mm(p.astype(BF), v_ref[t * KB:(t + 1) * KB, :])
            o = ot if o is None else o + ot
        return o

    def normalize(o, rows):
        l = l_buf[0, rows, :]
        for t in range(1, NKB):
            l = l + l_buf[t, rows, :]
        l = jnp.sum(l, axis=-1, keepdims=True)
        return (o * pltpu.reciprocal(l, full_range=False)).astype(BF)

    def stage_mod(h, slot):
        w = wm_buf[slot].astype(F32) * scol[...]
        mod_buf[h] = jnp.broadcast_to(jnp.sum(w, axis=0, keepdims=True), (8, 128))

    def head_step(h, slot):
        allr = slice(None)
        stage_mod(h, slot)
        q_buf[...] = stage_q(wq_buf.at[slot])
        o = stage_pv(allr, v_buf.at[slot])
        stage_s(q_buf[...], k_buf.at[slot])
        acc[...] = jnp.where(h > 0, acc[...], 0.0) + _mm(normalize(o, allr), wo_buf[slot])

    flag[0] = 1
    start_in_order(c_copy, *[x_copy(i) for i in range(NX)], wq0_copy, *[m1_copy(1, i) for i in range(M1C)],
                   *[m1_copy(0, i) for i in range(M1C)], cp_k(0, 1))

    c_copy.wait()
    cf = c_buf[...].astype(F32)
    sc = (cf * jax.nn.sigmoid(cf)).astype(BF)
    sc16 = jnp.broadcast_to(sc, (16, D))
    scf = sc.astype(F32)
    for j in range(KD):
        blk = jnp.broadcast_to(scf[:, j * 128:(j + 1) * 128], (128, 128))
        scol[j * 128:(j + 1) * 128, :] = blk.T

    for i in range(NX):
        x_copy(i).wait()
        for g in range(i * RX, (i + 1) * RX, RG):
            xf = x_buf[g:g + RG, :].astype(F32)
            d = xf - jnp.mean(xf, axis=-1, keepdims=True)
            acc[g:g + RG, :] = d * jax.lax.rsqrt(jnp.mean(d * d, axis=-1, keepdims=True) + EPS)

    def mod1(k):
        m = None
        for i in range(M1C):
            if k == 1:
                m1_copy(k, i).wait()
            elif i == 0:
                for ii in range(M1C):
                    m1_copy(k, ii).wait()
            t = _mm(sc16[:, i * MR:(i + 1) * MR], wm1_buf[k, i * MR:(i + 1) * MR, :])
            m = t if m is None else m + t
        return m[0:1, :].astype(BF).astype(F32)

    ca1 = (1.0 + mod1(1)).astype(BF).astype(F32)
    for cp in packet(0, 0):
        cp.start()
    wr_copy.start()
    wq0_copy.wait()
    q0 = None
    for j in range(KD):
        cols = slice(j * 128, (j + 1) * 128)
        hj = (acc[:, cols] * ca1[:, cols]).astype(BF)
        h_buf[j] = hj
        t = _mm(hj, wq0_buf[cols, :])
        q0 = t if q0 is None else q0 + t
    of_buf[...] = q0
    sa = mod1(0)
    cp_k(0, 1).wait()
    for j in range(KD):
        sa_col[j * 128:(j + 1) * 128, :] = jnp.broadcast_to(sa[:, j * 128:(j + 1) * 128], (128, 128)).T
    q_buf[...] = ((of_buf[...] + q_bias(wq0_buf)) * QSCALE).astype(BF)
    stage_s(q_buf[...], k_buf.at[1])

    def loop(h, carry):
        slot = h % 2

        @pl.when(h < FB)
        def _():
            for cp in moe_copies(h):
                cp.start()

        @pl.when(h < KD)
        def _():
            wd_copy(h).start()

        @pl.when(h + 2 < H)
        def _():
            cp_wq(h + 2, 1 - slot).start()
            cp_k(h + 2, 1 - slot).start()

        cp_v(h + 1, 1 - slot).start()
        cp_wm(h + 1, 1 - slot).start()
        cp_wo(h + 1, 1 - slot).start()
        for cp in packet(h, slot):
            cp.wait()
        head_step(h, slot)
        return carry

    jax.lax.fori_loop(0, H - 1, loop, 0)

    for cp in packet(H - 1, 1, last=True):
        cp.wait()
    wr_copy.wait()
    stage_mod(H - 1, 1)

    def mod_row(i):
        return jnp.concatenate([mod_buf[i * KD + j][0:1, :] for j in range(KD)], axis=1).astype(BF).astype(F32)

    cb1 = (1.0 + mod_row(2)).astype(BF).astype(F32)
    sb, gb = mod_row(1), mod_row(3)
    wr = wr_buf[...].astype(F32).reshape(1, D)
    for i, row in enumerate([mod_row(0), cb1 * wr, gb * cb1, gb * sb]):
        fin_buf[i] = jnp.broadcast_to(row, (8, D))
    r_const = jnp.sum(sb * wr, axis=-1, keepdims=True)

    def fin(i):
        return fin_buf[i][0:1, :]

    def last_pv(c):
        rows = pl.ds(c * RC, RC)
        of_buf[rows, :] = stage_pv(rows, v_buf.at[1])

    def last_o(c):
        rows = pl.ds(c * RC, RC)
        acc[rows, :] = acc[rows, :] + _mm(normalize(of_buf[rows, :], rows), wo_buf[1])

    def last_fin(c):
        for r0 in range(c * RC, (c + 1) * RC, 128):
            parts = []
            for g in range(r0, r0 + 128, RG):
                rows = slice(g, g + RG)
                x1 = x_buf[rows, :].astype(F32) + fin(0) * acc[rows, :]
                d = x1 - jnp.mean(x1, axis=-1, keepdims=True)
                rstd = jax.lax.rsqrt(jnp.mean(d * d, axis=-1, keepdims=True) + EPS)
                da = d * fin(1)
                part = da[:, 0:128]
                for j in range(1, KD):
                    part = part + da[:, j * 128:(j + 1) * 128]
                parts.append(part * rstd)
                o_stage[rows, :] = ((x1 + fin(3)) + (d * rstd) * fin(2)).astype(BF)
            blk = jnp.concatenate(parts, axis=0)
            r_buf[r0 // 128:r0 // 128 + 1, :] = jnp.sum(blk.T, axis=0, keepdims=True)
        out_copy(c * RC, c).start()

    for step in range(NC + 2):
        @pl.when(flag[0] == 1)
        def _():
            if 1 <= step <= NC:
                last_o(step - 1)
            if step < NC:
                last_pv(step)
            if step >= 2:
                last_fin(step - 2)

    rr = r_buf[...] + r_const
    row = (jax.lax.broadcasted_iota(jnp.int32, rr.shape, 0) * 128
           + jax.lax.broadcasted_iota(jnp.int32, rr.shape, 1))
    m1v = jnp.max(rr)
    i1 = jnp.clip(jnp.min(jnp.where(rr == m1v, row, S)), 0, S - 1)
    rr2 = jnp.where(row == i1, -jnp.inf, rr)
    m2v = jnp.max(rr2)
    i2 = jnp.clip(jnp.min(jnp.where(rr2 == m2v, row, S)), 0, S - 1)

    b1 = pl.multiple_of((i1 // 16) * 16, 16)
    b2 = pl.multiple_of((i2 // 16) * 16, 16)
    xs = (jnp.concatenate([x_buf[pl.ds(b1, 16), :], x_buf[pl.ds(b2, 16), :]], axis=0).astype(F32)
          + fin(0) * jnp.concatenate([acc[pl.ds(b1, 16), :], acc[pl.ds(b2, 16), :]], axis=0))
    h2 = _ln_mod(xs, cb1, sb).astype(BF)
    h2f = h2.astype(F32)

    for t, buf in enumerate((wg_buf, wu_buf, wd_buf)):
        pltpu.make_async_copy(buf, buf, sem_moe.at[t]).wait()
    acts = []
    for j in range(FB):
        g = _mm(h2, wg_buf[j])
        u = _mm(h2, wu_buf[j])
        acts.append((g * jax.nn.sigmoid(g) * u).astype(BF))
    ys = []
    for n in range(KD):
        y = None
        for j in range(FB):
            t = _mm(acts[j], wd_buf[n, j * 128:(j + 1) * 128, :])
            y = t if y is None else y + t
        ys.append(y)
    y = jnp.concatenate(ys, axis=1)
    g1 = jax.nn.sigmoid(jnp.full((1, 1), m1v, F32))
    g2 = jax.nn.sigmoid(jnp.full((1, 1), m2v, F32))
    row16 = jax.lax.broadcasted_iota(jnp.int32, (16, D), 0)

    for i in range(NC):
        out_copy(i * RC, i).wait()

    ya = y[0:16] * g1
    yb = y[16:32] * g2
    u1 = jnp.where(row16 == i1 - b1, ya, jnp.where(row16 == i2 - b1, yb, 0.0))
    u2 = jnp.where(row16 == i2 - b2, yb, jnp.where(row16 == i1 - b2, ya, 0.0))
    o_stage[pl.ds(b1, 16), :] = (xs[0:16] + gb * (h2f[0:16] + u1)).astype(BF)
    o_stage[pl.ds(b2, 16), :] = (xs[16:32] + gb * (h2f[16:32] + u2)).astype(BF)

    f1 = pltpu.make_async_copy(o_stage.at[pl.ds(b1, 16), :], out_hbm.at[pl.ds(b1, 16), :], sem_fix.at[0])
    f2 = pltpu.make_async_copy(o_stage.at[pl.ds(b2, 16), :], out_hbm.at[pl.ds(b2, 16), :], sem_fix.at[1])
    f1.start()

    @pl.when(b1 != b2)
    def _():
        f2.start()
        f2.wait()

    f1.wait()


@jax.jit
def pallas_adaLN_cond__mha_block_cached__moe_arch_mod__prompt_kernel(
    A_x: jax.Array,
    A_k_cache: jax.Array,
    A_v_cache: jax.Array,
    A_wq: jax.Array,
    A_wo: jax.Array,
    B_x: jax.Array,
    B_w_r: jax.Array,
    B_w_gate: jax.Array,
    B_w_up: jax.Array,
    B_w_down: jax.Array,
    c: jax.Array,
    w_mod: jax.Array,
):
    any_spec = pl.BlockSpec(memory_space=pl.ANY)
    out = pl.pallas_call(
        _kernel,
        out_shape=jax.ShapeDtypeStruct((S, D), BF),
        in_specs=[any_spec] * 11,
        out_specs=any_spec,
        scratch_shapes=[
            pltpu.VMEM((S, D), BF),
            pltpu.VMEM((S, D), BF),
            pltpu.VMEM((KD, S, 128), BF),
            pltpu.VMEM((S, D), F32),
            pltpu.VMEM((S, S), F32),
            pltpu.VMEM((S, 128), F32),
            pltpu.VMEM((S, 128), F32),
            pltpu.VMEM((NKB, S, 128), F32),
            pltpu.VMEM((S, DH), BF),
            pltpu.VMEM((2, S, DH), BF),
            pltpu.VMEM((2, S, DH), BF),
            pltpu.VMEM((2, D, DH), BF),
            pltpu.VMEM((2, DH, D), BF),
            pltpu.VMEM((2, D, 128), BF),
            pltpu.VMEM((D, DH), BF),
            pltpu.VMEM((2, D, D), BF),
            pltpu.VMEM((FB, D, 128), BF),
            pltpu.VMEM((FB, D, 128), BF),
            pltpu.VMEM((KD, F, 128), BF),
            pltpu.VMEM((1, D), BF),
            pltpu.VMEM((D,), BF),
            pltpu.VMEM((D, 128), F32),
            pltpu.VMEM((D, 128), F32),
            pltpu.VMEM((H, 8, 128), F32),
            pltpu.VMEM((5, 8, D), F32),
            pltpu.VMEM((S // 128, 128), F32),
            pltpu.SMEM((1,), jnp.int32),
            pltpu.SemaphoreType.DMA((2, 5)),
            pltpu.SemaphoreType.DMA((NX,)),
            pltpu.SemaphoreType.DMA((2, M1C)),
            pltpu.SemaphoreType.DMA((3,)),
            pltpu.SemaphoreType.DMA((3,)),
            pltpu.SemaphoreType.DMA((NC,)),
            pltpu.SemaphoreType.DMA((2,)),
            pltpu.SemaphoreType.REGULAR,
        ],
        compiler_params=pltpu.CompilerParams(vmem_limit_bytes=120 << 20, disable_bounds_checks=True),
    )(
        A_x.reshape(S, D),
        A_k_cache.reshape(H, S, DH),
        A_v_cache.reshape(H, S, DH),
        A_wq,
        A_wo,
        B_w_r,
        B_w_gate,
        B_w_up,
        B_w_down,
        c,
        w_mod,
    )
    return out.reshape(1, S, D)
```

```python
import jax
import jax.numpy as jnp
import jax.experimental.pallas as pl
import jax.experimental.pallas.tpu as pltpu

S = 2048
D = 1024
H = 32
DH = 128
F = 3584
KB = 512
NKB = S // KB
RX = 512
NX = S // RX
RG = 16
CH = ((0, 512), (512, 512), (1024, 512), (1536, 256), (1792, 256))
NC = len(CH)
KD = D // 128
FB = F // 128
M1C = 4
MR = D // M1C
EPS = 1e-5
LOG2E = 1.4426950408889634
QSCALE = (DH ** -0.5) * LOG2E
BF = jnp.bfloat16
F32 = jnp.float32


def _ln_mod(xf, mul, add):
    mu = jnp.mean(xf, axis=-1, keepdims=True)
    d = xf - mu
    var = jnp.mean(d * d, axis=-1, keepdims=True)
    return d * jax.lax.rsqrt(var + EPS) * mul + add


def _mm(a, b):
    return jnp.dot(a, b, preferred_element_type=F32)


def _kernel(x_hbm, k_hbm, v_hbm, wq_hbm, wo_hbm, wr_hbm, wg_hbm, wu_hbm, wd_hbm,
            c_hbm, wm_hbm, out_hbm,
            x_buf, o_stage, h_buf, acc, s_buf, m_buf, of_buf, l_buf,
            q_buf, k_buf, v_buf, wq_buf, wo_buf, wm_buf, wq0_buf,
            wm1_buf, wg_buf, wu_buf, wd_buf, c_buf, wr_buf, scol, sa_col, mod_buf, fin_buf, r_buf, flag,
            sem_pk, sem_x, sem_m1, sem_small, sem_moe, sem_out, sem_fix, sem_fence):
    def cp_k(h, slot):
        return pltpu.make_async_copy(k_hbm.at[h], k_buf.at[slot], sem_pk.at[slot, 0])

    def cp_v(h, slot):
        return pltpu.make_async_copy(v_hbm.at[h], v_buf.at[slot], sem_pk.at[slot, 1])

    def cp_wq(h, slot):
        return pltpu.make_async_copy(wq_hbm.at[:, pl.ds(h * DH, DH)], wq_buf.at[slot], sem_pk.at[slot, 2])

    def cp_wo(h, slot):
        return pltpu.make_async_copy(wo_hbm.at[pl.ds(h * DH, DH), :], wo_buf.at[slot], sem_pk.at[slot, 3])

    def cp_wm(h, slot):
        return pltpu.make_async_copy(wm_hbm.at[:, pl.ds(2 * D + h * 128, 128)], wm_buf.at[slot], sem_pk.at[slot, 4])

    def packet(h, slot, last=False):
        cps = [] if last else [cp_wq(h + 1, slot)]
        cps += [cp_v(h, slot), cp_wm(h, slot)]
        if not last:
            cps.append(cp_k(h + 1, slot))
        cps.append(cp_wo(h, slot))
        return cps

    def x_copy(i):
        rows = pl.ds(i * RX, RX)
        return pltpu.make_async_copy(x_hbm.at[rows, :], x_buf.at[rows, :], sem_x.at[i])

    def m1_copy(k, i):
        return pltpu.make_async_copy(wm_hbm.at[pl.ds(i * MR, MR), pl.ds(k * D, D)],
                                     wm1_buf.at[k, pl.ds(i * MR, MR), :], sem_m1.at[k, i])

    def moe_copies(j):
        return [
            pltpu.make_async_copy(wg_hbm.at[:, pl.ds(j * 128, 128)], wg_buf.at[j], sem_moe.at[0]),
            pltpu.make_async_copy(wu_hbm.at[:, pl.ds(j * 128, 128)], wu_buf.at[j], sem_moe.at[1]),
        ]

    def wd_copy(n):
        return pltpu.make_async_copy(wd_hbm.at[:, pl.ds(n * 128, 128)], wd_buf.at[n], sem_moe.at[2])

    def out_copy(i):
        rows = pl.ds(*CH[i])
        return pltpu.make_async_copy(o_stage.at[rows, :], out_hbm.at[rows, :], sem_out.at[i])

    c_copy = pltpu.make_async_copy(c_hbm, c_buf, sem_small.at[0])
    wr_copy = pltpu.make_async_copy(wr_hbm, wr_buf, sem_small.at[1])
    wq0_copy = pltpu.make_async_copy(wq_hbm.at[:, pl.ds(0, DH)], wq0_buf, sem_small.at[2])

    def start_in_order(*cps):
        for cp in cps:
            cp.start()
            pl.semaphore_signal(sem_fence, 1)
            pl.semaphore_wait(sem_fence, 1)

    def q_bias(wq):
        return jnp.sum(wq[...].astype(F32) * sa_col[...], axis=0, keepdims=True)

    def stage_q(wq):
        q = None
        for j in range(KD):
            t = _mm(h_buf[j], wq[j * 128:(j + 1) * 128, :])
            q = t if q is None else q + t
        return ((q + q_bias(wq)) * QSCALE).astype(BF)

    def qk_round(q, t, k_ref, rows, mx):
        s = jax.lax.dot_general(q, k_ref[t * KB:(t + 1) * KB, :], (((1,), (1,)), ((), ())),
                                preferred_element_type=F32)
        s_buf[rows, t * KB:(t + 1) * KB] = s
        for j in range(KB // 128):
            sj = s[:, j * 128:(j + 1) * 128]
            mx = sj if mx is None else jnp.maximum(mx, sj)
        return mx

    def row_max(mx):
        return jnp.broadcast_to(jnp.max(mx, axis=-1, keepdims=True), mx.shape)

    def stage_s(q, k_ref, rows=slice(None)):
        mx = None
        for t in range(NKB):
            mx = qk_round(q, t, k_ref, rows, mx)
        m_buf[rows, :] = row_max(mx)

    def stage_pv(rows, v_ref, b=0):
        m = m_buf[rows, :]
        m = jnp.concatenate([m] * (KB // 128), axis=1)
        o = None
        for t in range(NKB):
            p = jnp.exp2(s_buf[rows, t * KB:(t + 1) * KB] - m)
            l = p[:, 0:128]
            for j in range(1, KB // 128):
                l = l + p[:, j * 128:(j + 1) * 128]
            l_buf[b, t, rows, :] = l
            ot = _mm(p.astype(BF), v_ref[t * KB:(t + 1) * KB, :])
            o = ot if o is None else o + ot
        return o

    def normalize(o, rows, b=0):
        l = l_buf[b, 0, rows, :]
        for t in range(1, NKB):
            l = l + l_buf[b, t, rows, :]
        l = jnp.sum(l, axis=-1, keepdims=True)
        return (o * pltpu.reciprocal(l, full_range=False)).astype(BF)

    def stage_mod(h, slot):
        w = wm_buf[slot].astype(F32) * scol[...]
        mod_buf[h] = jnp.broadcast_to(jnp.sum(w, axis=0, keepdims=True), (8, 128))

    def head_step(h, slot):
        allr = slice(None)
        stage_mod(h, slot)
        q_buf[...] = stage_q(wq_buf.at[slot])
        o = stage_pv(allr, v_buf.at[slot])
        stage_s(q_buf[...], k_buf.at[slot])
        acc[...] = jnp.where(h > 0, acc[...], 0.0) + _mm(normalize(o, allr), wo_buf[slot])

    flag[0] = 1
    start_in_order(c_copy, *[x_copy(i) for i in range(NX)], wq0_copy, *[m1_copy(1, i) for i in range(M1C)],
                   *[m1_copy(0, i) for i in range(M1C)], cp_k(0, 1))

    c_copy.wait()
    cf = c_buf[...].astype(F32)
    sc = (cf * jax.nn.sigmoid(cf)).astype(BF)
    sc16 = jnp.broadcast_to(sc, (16, D))
    scf = sc.astype(F32)
    for j in range(KD):
        blk = jnp.broadcast_to(scf[:, j * 128:(j + 1) * 128], (128, 128))
        scol[j * 128:(j + 1) * 128, :] = blk.T

    for i in range(NX):
        x_copy(i).wait()
        for g in range(i * RX, (i + 1) * RX, RG):
            xf = x_buf[g:g + RG, :].astype(F32)
            d = xf - jnp.mean(xf, axis=-1, keepdims=True)
            acc[g:g + RG, :] = d * jax.lax.rsqrt(jnp.mean(d * d, axis=-1, keepdims=True) + EPS)

    def mod1(k):
        m = None
        for i in range(M1C):
            if k == 1:
                m1_copy(k, i).wait()
            elif i == 0:
                for ii in range(M1C):
                    m1_copy(k, ii).wait()
            t = _mm(sc16[:, i * MR:(i + 1) * MR], wm1_buf[k, i * MR:(i + 1) * MR, :])
            m = t if m is None else m + t
        return m[0:1, :].astype(BF).astype(F32)

    ca1 = (1.0 + mod1(1)).astype(BF).astype(F32)
    for cp in packet(0, 0):
        cp.start()
    wr_copy.start()
    wq0_copy.wait()
    q0 = None
    for j in range(KD):
        cols = slice(j * 128, (j + 1) * 128)
        hj = (acc[:, cols] * ca1[:, cols]).astype(BF)
        h_buf[j] = hj
        t = _mm(hj, wq0_buf[cols, :])
        q0 = t if q0 is None else q0 + t
    of_buf[0] = q0
    sa = mod1(0)
    cp_k(0, 1).wait()
    for j in range(KD):
        sa_col[j * 128:(j + 1) * 128, :] = jnp.broadcast_to(sa[:, j * 128:(j + 1) * 128], (128, 128)).T
    q_buf[...] = ((of_buf[0] + q_bias(wq0_buf)) * QSCALE).astype(BF)
    stage_s(q_buf[...], k_buf.at[1])

    def loop(h, carry):
        slot = h % 2

        @pl.when(h < FB)
        def _():
            for cp in moe_copies(h):
                cp.start()

        @pl.when(h < KD)
        def _():
            wd_copy(h).start()

        cp_wq(h + 2, 1 - slot).start()
        cp_k(h + 2, 1 - slot).start()
        cp_v(h + 1, 1 - slot).start()
        cp_wm(h + 1, 1 - slot).start()
        cp_wo(h + 1, 1 - slot).start()
        for cp in packet(h, slot):
            cp.wait()
        head_step(h, slot)
        return carry

    jax.lax.fori_loop(0, H - 2, loop, 0)

    for cp in packet(H - 1, 1, last=True):
        cp.start()
    for cp in packet(H - 2, 0):
        cp.wait()
    wr_copy.wait()
    stage_mod(H - 2, 0)
    q_buf[...] = stage_q(wq_buf.at[0])
    for cp in packet(H - 1, 1, last=True):
        cp.wait()
    stage_mod(H - 1, 1)

    def mod_row(i):
        return jnp.concatenate([mod_buf[i * KD + j][0:1, :] for j in range(KD)], axis=1).astype(BF).astype(F32)

    cb1 = (1.0 + mod_row(2)).astype(BF).astype(F32)
    sb, gb = mod_row(1), mod_row(3)
    wr = wr_buf[...].astype(F32).reshape(1, D)
    for i, row in enumerate([mod_row(0), cb1 * wr, gb * cb1, gb * sb]):
        fin_buf[i] = jnp.broadcast_to(row, (8, D))
    r_const = jnp.sum(sb * wr, axis=-1, keepdims=True)

    def fin(i):
        return fin_buf[i][0:1, :]

    def last_pv(c, b):
        rows = pl.ds(*CH[c])
        of_buf[b, rows, :] = stage_pv(rows, v_buf.at[b], b)

    def last_s(c):
        rows = pl.ds(*CH[c])
        stage_s(q_buf[rows, :], k_buf.at[0], rows)

    def last_o(c):
        rows = pl.ds(*CH[c])
        o2 = jnp.concatenate([normalize(of_buf[b, rows, :], rows, b) for b in range(2)], axis=1)
        wo2 = jnp.concatenate([wo_buf[0], wo_buf[1]], axis=0)
        acc[rows, :] = acc[rows, :] + _mm(o2, wo2)

    def last_fin(c):
        for r0 in range(CH[c][0], sum(CH[c]), 128):
            parts = []
            for g in range(r0, r0 + 128, RG):
                rows = slice(g, g + RG)
                x1 = x_buf[rows, :].astype(F32) + fin(0) * acc[rows, :]
                d = x1 - jnp.mean(x1, axis=-1, keepdims=True)
                rstd = jax.lax.rsqrt(jnp.mean(d * d, axis=-1, keepdims=True) + EPS)
                da = d * fin(1)
                part = da[:, 0:128]
                for j in range(1, KD):
                    part = part + da[:, j * 128:(j + 1) * 128]
                parts.append(part * rstd)
                o_stage[rows, :] = ((x1 + fin(3)) + (d * rstd) * fin(2)).astype(BF)
            blk = jnp.concatenate(parts, axis=0)
            r_buf[r0 // 128:r0 // 128 + 1, :] = jnp.sum(blk.T, axis=0, keepdims=True)
        out_copy(c).start()

    stages = (lambda c: last_pv(c, 0), last_s, lambda c: last_pv(c, 1), last_o, last_fin)
    for step in range(NC + len(stages) - 1):
        @pl.when(flag[0] == 1)
        def _():
            for lag in (2, 3, 0, 1, 4):
                if 0 <= step - lag < NC:
                    stages[lag](step - lag)

    rr = r_buf[...] + r_const
    row = (jax.lax.broadcasted_iota(jnp.int32, rr.shape, 0) * 128
           + jax.lax.broadcasted_iota(jnp.int32, rr.shape, 1))
    m1v = jnp.max(rr)
    i1 = jnp.clip(jnp.min(jnp.where(rr == m1v, row, S)), 0, S - 1)
    rr2 = jnp.where(row == i1, -jnp.inf, rr)
    m2v = jnp.max(rr2)
    i2 = jnp.clip(jnp.min(jnp.where(rr2 == m2v, row, S)), 0, S - 1)

    b1 = pl.multiple_of((i1 // 16) * 16, 16)
    b2 = pl.multiple_of((i2 // 16) * 16, 16)
    xs = (jnp.concatenate([x_buf[pl.ds(b1, 16), :], x_buf[pl.ds(b2, 16), :]], axis=0).astype(F32)
          + fin(0) * jnp.concatenate([acc[pl.ds(b1, 16), :], acc[pl.ds(b2, 16), :]], axis=0))
    h2 = _ln_mod(xs, cb1, sb).astype(BF)
    h2f = h2.astype(F32)

    for t, buf in enumerate((wg_buf, wu_buf, wd_buf)):
        pltpu.make_async_copy(buf, buf, sem_moe.at[t]).wait()
    acts = []
    for j in range(FB):
        g = _mm(h2, wg_buf[j])
        u = _mm(h2, wu_buf[j])
        acts.append((g * jax.nn.sigmoid(g) * u).astype(BF))
    ys = []
    for n in range(KD):
        y = None
        for j in range(FB):
            t = _mm(acts[j], wd_buf[n, j * 128:(j + 1) * 128, :])
            y = t if y is None else y + t
        ys.append(y)
    y = jnp.concatenate(ys, axis=1)
    g1 = jax.nn.sigmoid(jnp.full((1, 1), m1v, F32))
    g2 = jax.nn.sigmoid(jnp.full((1, 1), m2v, F32))
    row16 = jax.lax.broadcasted_iota(jnp.int32, (16, D), 0)

    for i in range(NC):
        out_copy(i).wait()

    ya = y[0:16] * g1
    yb = y[16:32] * g2
    u1 = jnp.where(row16 == i1 - b1, ya, jnp.where(row16 == i2 - b1, yb, 0.0))
    u2 = jnp.where(row16 == i2 - b2, yb, jnp.where(row16 == i1 - b2, ya, 0.0))
    o_stage[pl.ds(b1, 16), :] = (xs[0:16] + gb * (h2f[0:16] + u1)).astype(BF)
    o_stage[pl.ds(b2, 16), :] = (xs[16:32] + gb * (h2f[16:32] + u2)).astype(BF)

    f1 = pltpu.make_async_copy(o_stage.at[pl.ds(b1, 16), :], out_hbm.at[pl.ds(b1, 16), :], sem_fix.at[0])
    f2 = pltpu.make_async_copy(o_stage.at[pl.ds(b2, 16), :], out_hbm.at[pl.ds(b2, 16), :], sem_fix.at[1])
    f1.start()

    @pl.when(b1 != b2)
    def _():
        f2.start()
        f2.wait()

    f1.wait()


@jax.jit
def pallas_adaLN_cond__mha_block_cached__moe_arch_mod__prompt_kernel(
    A_x: jax.Array,
    A_k_cache: jax.Array,
    A_v_cache: jax.Array,
    A_wq: jax.Array,
    A_wo: jax.Array,
    B_x: jax.Array,
    B_w_r: jax.Array,
    B_w_gate: jax.Array,
    B_w_up: jax.Array,
    B_w_down: jax.Array,
    c: jax.Array,
    w_mod: jax.Array,
):
    any_spec = pl.BlockSpec(memory_space=pl.ANY)
    out = pl.pallas_call(
        _kernel,
        out_shape=jax.ShapeDtypeStruct((S, D), BF),
        in_specs=[any_spec] * 11,
        out_specs=any_spec,
        scratch_shapes=[
            pltpu.VMEM((S, D), BF),
            pltpu.VMEM((S, D), BF),
            pltpu.VMEM((KD, S, 128), BF),
            pltpu.VMEM((S, D), F32),
            pltpu.VMEM((S, S), F32),
            pltpu.VMEM((S, 128), F32),
            pltpu.VMEM((2, S, 128), F32),
            pltpu.VMEM((2, NKB, S, 128), F32),
            pltpu.VMEM((S, DH), BF),
            pltpu.VMEM((2, S, DH), BF),
            pltpu.VMEM((2, S, DH), BF),
            pltpu.VMEM((2, D, DH), BF),
            pltpu.VMEM((2, DH, D), BF),
            pltpu.VMEM((2, D, 128), BF),
            pltpu.VMEM((D, DH), BF),
            pltpu.VMEM((2, D, D), BF),
            pltpu.VMEM((FB, D, 128), BF),
            pltpu.VMEM((FB, D, 128), BF),
            pltpu.VMEM((KD, F, 128), BF),
            pltpu.VMEM((1, D), BF),
            pltpu.VMEM((D,), BF),
            pltpu.VMEM((D, 128), F32),
            pltpu.VMEM((D, 128), F32),
            pltpu.VMEM((H, 8, 128), F32),
            pltpu.VMEM((5, 8, D), F32),
            pltpu.VMEM((S // 128, 128), F32),
            pltpu.SMEM((1,), jnp.int32),
            pltpu.SemaphoreType.DMA((2, 5)),
            pltpu.SemaphoreType.DMA((NX,)),
            pltpu.SemaphoreType.DMA((2, M1C)),
            pltpu.SemaphoreType.DMA((3,)),
            pltpu.SemaphoreType.DMA((3,)),
            pltpu.SemaphoreType.DMA((NC,)),
            pltpu.SemaphoreType.DMA((2,)),
            pltpu.SemaphoreType.REGULAR,
        ],
        compiler_params=pltpu.CompilerParams(vmem_limit_bytes=120 << 20, disable_bounds_checks=True),
    )(
        A_x.reshape(S, D),
        A_k_cache.reshape(H, S, DH),
        A_v_cache.reshape(H, S, DH),
        A_wq,
        A_wo,
        B_w_r,
        B_w_gate,
        B_w_up,
        B_w_down,
        c,
        w_mod,
    )
    return out.reshape(1, S, D)
```

```python
import jax
import jax.numpy as jnp
import jax.experimental.pallas as pl
import jax.experimental.pallas.tpu as pltpu

S = 2048
D = 1024
H = 32
DH = 128
F = 3584
KB = 512
NKB = S // KB
RX = 512
NX = S // RX
RG = 16
CH = ((0, 512), (512, 512), (1024, 512), (1536, 256), (1792, 256))
NC = len(CH)
KD = D // 128
FB = F // 128
M1C = 4
MR = D // M1C
EPS = 1e-5
LOG2E = 1.4426950408889634
QSCALE = (DH ** -0.5) * LOG2E
BF = jnp.bfloat16
F32 = jnp.float32


def _ln_mod(xf, mul, add):
    mu = jnp.mean(xf, axis=-1, keepdims=True)
    d = xf - mu
    var = jnp.mean(d * d, axis=-1, keepdims=True)
    return d * jax.lax.rsqrt(var + EPS) * mul + add


def _mm(a, b):
    return jnp.dot(a, b, preferred_element_type=F32)


def _kernel(x_hbm, k_hbm, v_hbm, wq_hbm, wo_hbm, wr_hbm, wg_hbm, wu_hbm, wd_hbm,
            c_hbm, wm_hbm, out_hbm,
            x_buf, o_stage, h_buf, acc, s_buf, m_buf, of_buf, l_buf,
            q_buf, k_buf, v_buf, wq_buf, wo_buf, wm_buf, wq0_buf,
            wm1_buf, wg_buf, wu_buf, wd_buf, c_buf, wr_buf, scol, sa_col, mod_buf, fin_buf, r_buf, flag,
            sem_pk, sem_x, sem_m1, sem_small, sem_moe, sem_out, sem_fix, sem_fence):
    def cp_k(h, slot):
        return pltpu.make_async_copy(k_hbm.at[h], k_buf.at[slot], sem_pk.at[slot, 0])

    def cp_v(h, slot):
        return pltpu.make_async_copy(v_hbm.at[h], v_buf.at[slot], sem_pk.at[slot, 1])

    def cp_wq(h, slot):
        return pltpu.make_async_copy(wq_hbm.at[:, pl.ds(h * DH, DH)], wq_buf.at[slot], sem_pk.at[slot, 2])

    def cp_wo(h, slot):
        return pltpu.make_async_copy(wo_hbm.at[pl.ds(h * DH, DH), :], wo_buf.at[slot], sem_pk.at[slot, 3])

    def cp_wm(h, slot):
        return pltpu.make_async_copy(wm_hbm.at[:, pl.ds(2 * D + h * 128, 128)], wm_buf.at[slot], sem_pk.at[slot, 4])

    def packet(h, slot, last=False):
        cps = [] if last else [cp_wq(h + 1, slot)]
        cps += [cp_v(h, slot), cp_wm(h, slot)]
        if not last:
            cps.append(cp_k(h + 1, slot))
        cps.append(cp_wo(h, slot))
        return cps

    def x_copy(i):
        rows = pl.ds(i * RX, RX)
        return pltpu.make_async_copy(x_hbm.at[rows, :], x_buf.at[rows, :], sem_x.at[i])

    def m1_copy(k, i):
        return pltpu.make_async_copy(wm_hbm.at[pl.ds(i * MR, MR), pl.ds(k * D, D)],
                                     wm1_buf.at[k, pl.ds(i * MR, MR), :], sem_m1.at[k, i])

    def moe_copies(j):
        return [
            pltpu.make_async_copy(wg_hbm.at[:, pl.ds(j * 128, 128)], wg_buf.at[j], sem_moe.at[0]),
            pltpu.make_async_copy(wu_hbm.at[:, pl.ds(j * 128, 128)], wu_buf.at[j], sem_moe.at[1]),
        ]

    def wd_copy(n):
        return pltpu.make_async_copy(wd_hbm.at[:, pl.ds(n * 128, 128)], wd_buf.at[n], sem_moe.at[2])

    def out_copy(i):
        rows = pl.ds(*CH[i])
        return pltpu.make_async_copy(o_stage.at[rows, :], out_hbm.at[rows, :], sem_out.at[i])

    c_copy = pltpu.make_async_copy(c_hbm, c_buf, sem_small.at[0])
    wr_copy = pltpu.make_async_copy(wr_hbm, wr_buf, sem_small.at[1])
    wq0_copy = pltpu.make_async_copy(wq_hbm.at[:, pl.ds(0, DH)], wq0_buf, sem_small.at[2])

    def start_in_order(*cps):
        for cp in cps:
            cp.start()
            pl.semaphore_signal(sem_fence, 1)
            pl.semaphore_wait(sem_fence, 1)

    def q_bias(wq):
        return jnp.sum(wq[...].astype(F32) * sa_col[...], axis=0, keepdims=True)

    def stage_q(wq):
        q = None
        for j in range(KD):
            t = _mm(h_buf[j], wq[j * 128:(j + 1) * 128, :])
            q = t if q is None else q + t
        return ((q + q_bias(wq)) * QSCALE).astype(BF)

    def qk_round(q, t, k_ref, rows, mx):
        s = jax.lax.dot_general(q, k_ref[t * KB:(t + 1) * KB, :], (((1,), (1,)), ((), ())),
                                preferred_element_type=F32)
        s_buf[rows, t * KB:(t + 1) * KB] = s
        for j in range(KB // 128):
            sj = s[:, j * 128:(j + 1) * 128]
            mx = sj if mx is None else jnp.maximum(mx, sj)
        return mx

    def row_max(mx):
        return jnp.broadcast_to(jnp.max(mx, axis=-1, keepdims=True), mx.shape)

    def stage_s(q, k_ref, rows=slice(None)):
        mx = None
        for t in range(NKB):
            mx = qk_round(q, t, k_ref, rows, mx)
        m_buf[rows, :] = row_max(mx)

    def stage_pv(rows, v_ref, b=0):
        m = m_buf[rows, :]
        m = jnp.concatenate([m] * (KB // 128), axis=1)
        o = None
        for t in range(NKB):
            p = jnp.exp2(s_buf[rows, t * KB:(t + 1) * KB] - m)
            l = p[:, 0:128]
            for j in range(1, KB // 128):
                l = l + p[:, j * 128:(j + 1) * 128]
            l_buf[b, t, rows, :] = l
            ot = _mm(p.astype(BF), v_ref[t * KB:(t + 1) * KB, :])
            o = ot if o is None else o + ot
        return o

    def normalize(o, rows, b=0):
        l = l_buf[b, 0, rows, :]
        for t in range(1, NKB):
            l = l + l_buf[b, t, rows, :]
        l = jnp.sum(l, axis=-1, keepdims=True)
        return (o * pltpu.reciprocal(l, full_range=False)).astype(BF)

    def stage_mod(h, slot):
        w = wm_buf[slot].astype(F32) * scol[...]
        mod_buf[h] = jnp.broadcast_to(jnp.sum(w, axis=0, keepdims=True), (8, 128))

    def head_step(h, slot):
        allr = slice(None)
        stage_mod(h, slot)
        q_buf[...] = stage_q(wq_buf.at[slot])
        o = stage_pv(allr, v_buf.at[slot])
        stage_s(q_buf[...], k_buf.at[slot])
        acc[...] = jnp.where(h > 0, acc[...], 0.0) + _mm(normalize(o, allr), wo_buf[slot])

    flag[0] = 1
    start_in_order(c_copy, *[x_copy(i) for i in range(NX)], wq0_copy, *[m1_copy(1, i) for i in range(M1C)],
                   *[m1_copy(0, i) for i in range(M1C)], cp_k(0, 1))

    c_copy.wait()
    cf = c_buf[...].astype(F32)
    sc = (cf * jax.nn.sigmoid(cf)).astype(BF)
    sc16 = jnp.broadcast_to(sc, (16, D))
    scf = sc.astype(F32)
    for j in range(KD):
        blk = jnp.broadcast_to(scf[:, j * 128:(j + 1) * 128], (128, 128))
        scol[j * 128:(j + 1) * 128, :] = blk.T

    for i in range(NX):
        x_copy(i).wait()
        for g in range(i * RX, (i + 1) * RX, RG):
            xf = x_buf[g:g + RG, :].astype(F32)
            mu = jnp.mean(xf, axis=-1, keepdims=True)
            d = xf - mu
            acc[g:g + RG, :] = d * jax.lax.rsqrt(jnp.mean(d * d, axis=-1, keepdims=True) + EPS)

    def mod1(k):
        m = None
        for i in range(M1C):
            if k == 1:
                m1_copy(k, i).wait()
            elif i == 0:
                for ii in range(M1C):
                    m1_copy(k, ii).wait()
            t = _mm(sc16[:, i * MR:(i + 1) * MR], wm1_buf[k, i * MR:(i + 1) * MR, :])
            m = t if m is None else m + t
        return m[0:1, :].astype(BF).astype(F32)

    ca1 = (1.0 + mod1(1)).astype(BF).astype(F32)
    for cp in packet(0, 0):
        cp.start()
    wr_copy.start()
    wq0_copy.wait()
    q0 = None
    for j in range(KD):
        cols = slice(j * 128, (j + 1) * 128)
        hj = (acc[:, cols] * ca1[:, cols]).astype(BF)
        h_buf[j] = hj
        t = _mm(hj, wq0_buf[cols, :])
        q0 = t if q0 is None else q0 + t
    of_buf[0] = q0
    sa = mod1(0)
    cp_k(0, 1).wait()
    for j in range(KD):
        sa_col[j * 128:(j + 1) * 128, :] = jnp.broadcast_to(sa[:, j * 128:(j + 1) * 128], (128, 128)).T
    q_buf[...] = ((of_buf[0] + q_bias(wq0_buf)) * QSCALE).astype(BF)
    stage_s(q_buf[...], k_buf.at[1])

    def loop(h, carry):
        slot = h & 1
        for cp in packet(h, slot):
            cp.wait()

        @pl.when(h < FB)
        def _():
            for cp in moe_copies(h):
                cp.start()

        @pl.when(h < KD)
        def _():
            wd_copy(h).start()

        cp_wq(h + 2, 1 - slot).start()
        cp_k(h + 2, 1 - slot).start()
        cp_v(h + 1, 1 - slot).start()
        cp_wm(h + 1, 1 - slot).start()
        cp_wo(h + 1, 1 - slot).start()
        head_step(h, slot)
        return carry

    jax.lax.fori_loop(0, H - 2, loop, 0)

    for cp in packet(H - 1, 1, last=True):
        cp.start()
    for cp in packet(H - 2, 0):
        cp.wait()
    wr_copy.wait()
    stage_mod(H - 2, 0)
    q_buf[...] = stage_q(wq_buf.at[0])
    rows0 = pl.ds(*CH[0])
    of_buf[0, rows0, :] = stage_pv(rows0, v_buf.at[0])
    for cp in packet(H - 1, 1, last=True):
        cp.wait()

    def mod_row(i):
        return jnp.concatenate([mod_buf[i * KD + j][0:1, :] for j in range(KD)], axis=1).astype(BF).astype(F32)

    def fin_consts():
        stage_mod(H - 1, 1)
        cb1 = (1.0 + mod_row(2)).astype(BF).astype(F32)
        sb, gb = mod_row(1), mod_row(3)
        wr = wr_buf[...].astype(F32).reshape(1, D)
        for i, row in enumerate([mod_row(0), cb1 * wr, gb * cb1, gb * sb, cb1, sb, gb, wr]):
            fin_buf[i] = jnp.broadcast_to(row, (8, D))

    def fin(i):
        return fin_buf[i][0:1, :]

    def last_pv(c, b):
        rows = pl.ds(*CH[c])
        of_buf[b, rows, :] = stage_pv(rows, v_buf.at[b], b)

    def last_s(c):
        rows = pl.ds(*CH[c])
        stage_s(q_buf[rows, :], k_buf.at[0], rows)

    def last_o(c):
        rows = pl.ds(*CH[c])
        o2 = jnp.concatenate([normalize(of_buf[b, rows, :], rows, b) for b in range(2)], axis=1)
        wo2 = jnp.concatenate([wo_buf[0], wo_buf[1]], axis=0)
        acc[rows, :] = acc[rows, :] + _mm(o2, wo2)

    def last_fin(c):
        for r0 in range(CH[c][0], sum(CH[c]), 128):
            parts = []
            for g in range(r0, r0 + 128, RG):
                rows = slice(g, g + RG)
                x1 = x_buf[rows, :].astype(F32) + fin(0) * acc[rows, :]
                d = x1 - jnp.mean(x1, axis=-1, keepdims=True)
                rstd = jax.lax.rsqrt(jnp.mean(d * d, axis=-1, keepdims=True) + EPS)
                da = d * fin(1)
                part = da[:, 0:128]
                for j in range(1, KD):
                    part = part + da[:, j * 128:(j + 1) * 128]
                parts.append(part * rstd)
                o_stage[rows, :] = ((x1 + fin(3)) + (d * rstd) * fin(2)).astype(BF)
            blk = jnp.concatenate(parts, axis=0)
            r_buf[r0 // 128:r0 // 128 + 1, :] = jnp.sum(blk.T, axis=0, keepdims=True)
        out_copy(c).start()

    stages = (lambda c: last_pv(c, 0), last_s, lambda c: last_pv(c, 1), last_o, last_fin)
    for step in range(1, NC + len(stages) - 2):
        @pl.when(flag[0] == 1)
        def _():
            if step == 1:
                fin_consts()
            for lag in (2, 3, 0, 1, 4):
                if 0 <= step - lag < NC:
                    stages[lag](step - lag)
            if step == NC + 2:
                last_fin(NC - 1)

    ga, cb1, sb, gb = fin(0), fin(4), fin(5), fin(6)
    rr = r_buf[...] + jnp.sum(sb * fin(7), axis=-1, keepdims=True)
    row = (jax.lax.broadcasted_iota(jnp.int32, rr.shape, 0) * 128
           + jax.lax.broadcasted_iota(jnp.int32, rr.shape, 1))

    def top1(v):
        m = jnp.max(jnp.max(v, axis=0, keepdims=True), axis=1, keepdims=True)
        i = jnp.min(jnp.min(jnp.where(v == m, row, S - 1), axis=0, keepdims=True), axis=1, keepdims=True)
        return m, i

    m1v, i1v = top1(rr)
    m2v, i2v = top1(jnp.where(row == i1v, -jnp.inf, rr))
    i1, i2 = i1v[0, 0], i2v[0, 0]

    b1 = pl.multiple_of((i1 // 16) * 16, 16)
    b2 = pl.multiple_of((i2 // 16) * 16, 16)
    xs = (jnp.concatenate([x_buf[pl.ds(b1, 16), :], x_buf[pl.ds(b2, 16), :]], axis=0).astype(F32)
          + ga * jnp.concatenate([acc[pl.ds(b1, 16), :], acc[pl.ds(b2, 16), :]], axis=0))
    h2 = _ln_mod(xs, cb1, sb).astype(BF)
    h2f = h2.astype(F32)

    for t, buf in enumerate((wg_buf, wu_buf, wd_buf)):
        pltpu.make_async_copy(buf, buf, sem_moe.at[t]).wait()
    acts = []
    for j in range(FB):
        g = _mm(h2, wg_buf[j])
        u = _mm(h2, wu_buf[j])
        acts.append((g * jax.nn.sigmoid(g) * u).astype(BF))
    ys = []
    for n in range(KD):
        y = None
        for j in range(FB):
            t = _mm(acts[j], wd_buf[n, j * 128:(j + 1) * 128, :])
            y = t if y is None else y + t
        ys.append(y)
    y = jnp.concatenate(ys, axis=1)
    g1 = jax.nn.sigmoid(m1v)
    g2 = jax.nn.sigmoid(m2v)
    row16 = jax.lax.broadcasted_iota(jnp.int32, (16, D), 0)

    for i in range(NC):
        out_copy(i).wait()

    ya = y[0:16] * g1
    yb = y[16:32] * g2
    u1 = jnp.where(row16 == i1 - b1, ya, jnp.where(row16 == i2 - b1, yb, 0.0))
    u2 = jnp.where(row16 == i2 - b2, yb, jnp.where(row16 == i1 - b2, ya, 0.0))
    o_stage[pl.ds(b1, 16), :] = (xs[0:16] + gb * (h2f[0:16] + u1)).astype(BF)
    o_stage[pl.ds(b2, 16), :] = (xs[16:32] + gb * (h2f[16:32] + u2)).astype(BF)

    f1 = pltpu.make_async_copy(o_stage.at[pl.ds(b1, 16), :], out_hbm.at[pl.ds(b1, 16), :], sem_fix.at[0])
    f2 = pltpu.make_async_copy(o_stage.at[pl.ds(b2, 16), :], out_hbm.at[pl.ds(b2, 16), :], sem_fix.at[1])
    f1.start()

    @pl.when(b1 != b2)
    def _():
        f2.start()
        f2.wait()

    f1.wait()


@jax.jit
def pallas_adaLN_cond__mha_block_cached__moe_arch_mod__prompt_kernel(
    A_x: jax.Array,
    A_k_cache: jax.Array,
    A_v_cache: jax.Array,
    A_wq: jax.Array,
    A_wo: jax.Array,
    B_x: jax.Array,
    B_w_r: jax.Array,
    B_w_gate: jax.Array,
    B_w_up: jax.Array,
    B_w_down: jax.Array,
    c: jax.Array,
    w_mod: jax.Array,
):
    any_spec = pl.BlockSpec(memory_space=pl.ANY)
    out = pl.pallas_call(
        _kernel,
        out_shape=jax.ShapeDtypeStruct((S, D), BF),
        in_specs=[any_spec] * 11,
        out_specs=any_spec,
        scratch_shapes=[
            pltpu.VMEM((S, D), BF),
            pltpu.VMEM((S, D), BF),
            pltpu.VMEM((KD, S, 128), BF),
            pltpu.VMEM((S, D), F32),
            pltpu.VMEM((S, S), F32),
            pltpu.VMEM((S, 128), F32),
            pltpu.VMEM((2, S, 128), F32),
            pltpu.VMEM((2, NKB, S, 128), F32),
            pltpu.VMEM((S, DH), BF),
            pltpu.VMEM((2, S, DH), BF),
            pltpu.VMEM((2, S, DH), BF),
            pltpu.VMEM((2, D, DH), BF),
            pltpu.VMEM((2, DH, D), BF),
            pltpu.VMEM((2, D, 128), BF),
            pltpu.VMEM((D, DH), BF),
            pltpu.VMEM((2, D, D), BF),
            pltpu.VMEM((FB, D, 128), BF),
            pltpu.VMEM((FB, D, 128), BF),
            pltpu.VMEM((KD, F, 128), BF),
            pltpu.VMEM((1, D), BF),
            pltpu.VMEM((D,), BF),
            pltpu.VMEM((D, 128), F32),
            pltpu.VMEM((D, 128), F32),
            pltpu.VMEM((H, 8, 128), F32),
            pltpu.VMEM((8, 8, D), F32),
            pltpu.VMEM((S // 128, 128), F32),
            pltpu.SMEM((1,), jnp.int32),
            pltpu.SemaphoreType.DMA((2, 5)),
            pltpu.SemaphoreType.DMA((NX,)),
            pltpu.SemaphoreType.DMA((2, M1C)),
            pltpu.SemaphoreType.DMA((3,)),
            pltpu.SemaphoreType.DMA((3,)),
            pltpu.SemaphoreType.DMA((NC,)),
            pltpu.SemaphoreType.DMA((2,)),
            pltpu.SemaphoreType.REGULAR,
        ],
        compiler_params=pltpu.CompilerParams(vmem_limit_bytes=120 << 20, disable_bounds_checks=True),
    )(
        A_x.reshape(S, D),
        A_k_cache.reshape(H, S, DH),
        A_v_cache.reshape(H, S, DH),
        A_wq,
        A_wo,
        B_w_r,
        B_w_gate,
        B_w_up,
        B_w_down,
        c,
        w_mod,
    )
    return out.reshape(1, S, D)
```

```python
import jax
import jax.numpy as jnp
import jax.experimental.pallas as pl
import jax.experimental.pallas.tpu as pltpu

S = 2048
D = 1024
H = 32
DH = 128
F = 3584
KB = 512
NKB = S // KB
RX = 512
NX = S // RX
RG = 16
CH = ((0, 512), (512, 512), (1024, 512), (1536, 256), (1792, 256))
NC = len(CH)
KD = D // 128
FB = F // 128
M1C = 4
MR = D // M1C
EPS = 1e-5
LOG2E = 1.4426950408889634
QSCALE = (DH ** -0.5) * LOG2E
BF = jnp.bfloat16
F32 = jnp.float32


def _ln_mod(xf, mul, add):
    mu = jnp.mean(xf, axis=-1, keepdims=True)
    d = xf - mu
    var = jnp.mean(d * d, axis=-1, keepdims=True)
    return d * jax.lax.rsqrt(var + EPS) * mul + add


def _mm(a, b):
    return jnp.dot(a, b, preferred_element_type=F32)


def _kernel(x_hbm, k_hbm, v_hbm, wq_hbm, wo_hbm, wr_hbm, wg_hbm, wu_hbm, wd_hbm,
            c_hbm, wm_hbm, out_hbm,
            x_buf, o_stage, h_buf, acc, s_buf, m_buf, of_buf, l_buf,
            q_buf, pk_buf, wo_buf, wq0_buf,
            wm1_buf, wg_buf, wu_buf, wd_buf, c_buf, wr_buf, scol, sa_col, mod_buf, fin_buf, r_buf, flag,
            sem_pk, sem_wo, sem_x, sem_m1, sem_small, sem_moe, sem_out, sem_fix, sem_fence):
    def k_buf(slot):
        return pk_buf.at[slot, pl.ds(0, S), :]

    def wq_buf(slot):
        return pk_buf.at[slot, pl.ds(S, D), :]

    def v_buf(slot):
        return pk_buf.at[slot, pl.ds(S + D, S), :]

    def wm_buf(slot):
        return pk_buf.at[slot, pl.ds(2 * S + D, D), :]

    def cp_k(h, slot):
        return pltpu.make_async_copy(k_hbm.at[h], k_buf(slot), sem_pk.at[slot])

    def cp_v(h, slot):
        return pltpu.make_async_copy(v_hbm.at[h], v_buf(slot), sem_pk.at[slot])

    def cp_wq(h, slot):
        return pltpu.make_async_copy(wq_hbm.at[:, pl.ds(h * DH, DH)], wq_buf(slot), sem_pk.at[slot])

    def cp_wm(h, slot):
        return pltpu.make_async_copy(wm_hbm.at[:, pl.ds(2 * D + h * 128, 128)], wm_buf(slot), sem_pk.at[slot])

    def cp_wo(h, slot):
        return pltpu.make_async_copy(wo_hbm.at[pl.ds(h * DH, DH), :], wo_buf.at[slot], sem_wo.at[slot])

    def wait_packet(slot, last=False):
        dst = pk_buf.at[slot, pl.ds(S + D, S + D), :] if last else pk_buf.at[slot]
        pltpu.make_async_copy(dst, dst, sem_pk.at[slot]).wait()
        cp_wo(0, slot).wait()

    def packet(h, slot, last=False):
        cps = [] if last else [cp_wq(h + 1, slot)]
        cps += [cp_v(h, slot), cp_wm(h, slot)]
        if not last:
            cps.append(cp_k(h + 1, slot))
        cps.append(cp_wo(h, slot))
        return cps

    def x_copy(i):
        rows = pl.ds(i * RX, RX)
        return pltpu.make_async_copy(x_hbm.at[rows, :], x_buf.at[rows, :], sem_x.at[i])

    def m1_copy(k, i):
        return pltpu.make_async_copy(wm_hbm.at[pl.ds(i * MR, MR), pl.ds(k * D, D)],
                                     wm1_buf.at[k, pl.ds(i * MR, MR), :], sem_m1.at[k, i])

    def moe_copies(j):
        return [
            pltpu.make_async_copy(wg_hbm.at[:, pl.ds(j * 128, 128)], wg_buf.at[j], sem_moe.at[0]),
            pltpu.make_async_copy(wu_hbm.at[:, pl.ds(j * 128, 128)], wu_buf.at[j], sem_moe.at[1]),
        ]

    def wd_copy(n):
        return pltpu.make_async_copy(wd_hbm.at[:, pl.ds(n * 128, 128)], wd_buf.at[n], sem_moe.at[2])

    def out_copy(i):
        rows = pl.ds(*CH[i])
        return pltpu.make_async_copy(o_stage.at[rows, :], out_hbm.at[rows, :], sem_out.at[i])

    c_copy = pltpu.make_async_copy(c_hbm, c_buf, sem_small.at[0])
    wr_copy = pltpu.make_async_copy(wr_hbm, wr_buf, sem_small.at[1])
    wq0_copy = pltpu.make_async_copy(wq_hbm.at[:, pl.ds(0, DH)], wq0_buf, sem_small.at[2])

    def start_in_order(*cps):
        for cp in cps:
            cp.start()
            pl.semaphore_signal(sem_fence, 1)
            pl.semaphore_wait(sem_fence, 1)

    def q_bias(wq):
        return jnp.sum(wq[...].astype(F32) * sa_col[...], axis=0, keepdims=True)

    def stage_q(wq):
        q = None
        for j in range(KD):
            t = _mm(h_buf[j], wq[j * 128:(j + 1) * 128, :])
            q = t if q is None else q + t
        return ((q + q_bias(wq)) * QSCALE).astype(BF)

    def qk_round(q, t, k_ref, rows, mx):
        s = jax.lax.dot_general(q, k_ref[t * KB:(t + 1) * KB, :], (((1,), (1,)), ((), ())),
                                preferred_element_type=F32)
        s_buf[rows, t * KB:(t + 1) * KB] = s
        for j in range(KB // 128):
            sj = s[:, j * 128:(j + 1) * 128]
            mx = sj if mx is None else jnp.maximum(mx, sj)
        return mx

    def row_max(mx):
        return jnp.broadcast_to(jnp.max(mx, axis=-1, keepdims=True), mx.shape)

    def stage_s(q, k_ref, rows=slice(None)):
        mx = None
        for t in range(NKB):
            mx = qk_round(q, t, k_ref, rows, mx)
        m_buf[rows, :] = row_max(mx)

    def stage_pv(rows, v_ref, b=0):
        m = m_buf[rows, :]
        m = jnp.concatenate([m] * (KB // 128), axis=1)
        o = None
        for t in range(NKB):
            p = jnp.exp2(s_buf[rows, t * KB:(t + 1) * KB] - m)
            l = p[:, 0:128]
            for j in range(1, KB // 128):
                l = l + p[:, j * 128:(j + 1) * 128]
            l_buf[b, t, rows, :] = l
            ot = _mm(p.astype(BF), v_ref[t * KB:(t + 1) * KB, :])
            o = ot if o is None else o + ot
        return o

    def normalize(o, rows, b=0):
        l = l_buf[b, 0, rows, :]
        for t in range(1, NKB):
            l = l + l_buf[b, t, rows, :]
        l = jnp.sum(l, axis=-1, keepdims=True)
        return (o * pltpu.reciprocal(l, full_range=False)).astype(BF)

    def stage_mod(h, slot):
        w = wm_buf(slot)[...].astype(F32) * scol[...]
        mod_buf[h] = jnp.broadcast_to(jnp.sum(w, axis=0, keepdims=True), (8, 128))

    def head_step(h, slot):
        allr = slice(None)
        stage_mod(h, slot)
        q_buf[...] = stage_q(wq_buf(slot))
        o = stage_pv(allr, v_buf(slot))
        stage_s(q_buf[...], k_buf(slot))
        acc[...] = jnp.where(h > 0, acc[...], 0.0) + _mm(normalize(o, allr), wo_buf[slot])

    flag[0] = 1
    start_in_order(c_copy, *[x_copy(i) for i in range(NX)], wq0_copy, *[m1_copy(1, i) for i in range(M1C)],
                   *[m1_copy(0, i) for i in range(M1C)], cp_k(0, 1))

    c_copy.wait()
    cf = c_buf[...].astype(F32)
    sc = (cf * jax.nn.sigmoid(cf)).astype(BF)
    sc16 = jnp.broadcast_to(sc, (16, D))
    scf = sc.astype(F32)
    for j in range(KD):
        blk = jnp.broadcast_to(scf[:, j * 128:(j + 1) * 128], (128, 128))
        scol[j * 128:(j + 1) * 128, :] = blk.T

    for i in range(NX):
        x_copy(i).wait()
        for g in range(i * RX, (i + 1) * RX, RG):
            xf = x_buf[g:g + RG, :].astype(F32)
            mu = jnp.mean(xf, axis=-1, keepdims=True)
            d = xf - mu
            acc[g:g + RG, :] = d * jax.lax.rsqrt(jnp.mean(d * d, axis=-1, keepdims=True) + EPS)

    def mod1(k):
        m = None
        for i in range(M1C):
            if k == 1:
                m1_copy(k, i).wait()
            elif i == 0:
                for ii in range(M1C):
                    m1_copy(k, ii).wait()
            t = _mm(sc16[:, i * MR:(i + 1) * MR], wm1_buf[k, i * MR:(i + 1) * MR, :])
            m = t if m is None else m + t
        return m[0:1, :].astype(BF).astype(F32)

    ca1 = (1.0 + mod1(1)).astype(BF).astype(F32)
    for cp in packet(0, 0):
        cp.start()
    wr_copy.start()
    wq0_copy.wait()
    q0 = None
    for j in range(KD):
        cols = slice(j * 128, (j + 1) * 128)
        hj = (acc[:, cols] * ca1[:, cols]).astype(BF)
        h_buf[j] = hj
        t = _mm(hj, wq0_buf[cols, :])
        q0 = t if q0 is None else q0 + t
    of_buf[0] = q0
    sa = mod1(0)
    cp_k(0, 1).wait()
    for j in range(KD):
        sa_col[j * 128:(j + 1) * 128, :] = jnp.broadcast_to(sa[:, j * 128:(j + 1) * 128], (128, 128)).T
    bias = _mm(jnp.broadcast_to(sa, (16, D)).astype(BF), wq0_buf[...])[0:1, :]
    q_buf[...] = ((of_buf[0] + bias) * QSCALE).astype(BF)
    stage_s(q_buf[...], k_buf(1))

    def loop(h, carry):
        slot = h & 1
        wait_packet(slot)

        @pl.when(h < FB)
        def _():
            for cp in moe_copies(h):
                cp.start()

        @pl.when(h < KD)
        def _():
            wd_copy(h).start()

        cp_wq(h + 2, 1 - slot).start()
        cp_k(h + 2, 1 - slot).start()
        cp_v(h + 1, 1 - slot).start()
        cp_wm(h + 1, 1 - slot).start()
        cp_wo(h + 1, 1 - slot).start()
        head_step(h, slot)
        return carry

    jax.lax.fori_loop(0, H - 2, loop, 0)

    for cp in packet(H - 1, 1, last=True):
        cp.start()
    wait_packet(0)
    wr_copy.wait()
    stage_mod(H - 2, 0)
    q_buf[...] = stage_q(wq_buf(0))
    rows0 = pl.ds(*CH[0])
    of_buf[0, rows0, :] = stage_pv(rows0, v_buf(0))
    wait_packet(1, last=True)

    def mod_row(i):
        return jnp.concatenate([mod_buf[i * KD + j][0:1, :] for j in range(KD)], axis=1).astype(BF).astype(F32)

    def fin_consts():
        stage_mod(H - 1, 1)
        cb1 = (1.0 + mod_row(2)).astype(BF).astype(F32)
        sb, gb = mod_row(1), mod_row(3)
        wr = wr_buf[...].astype(F32).reshape(1, D)
        for i, row in enumerate([mod_row(0), cb1 * wr, gb * cb1, gb * sb, cb1, sb, gb, wr]):
            fin_buf[i] = jnp.broadcast_to(row, (8, D))

    def fin(i):
        return fin_buf[i][0:1, :]

    def last_pv(c, b):
        rows = pl.ds(*CH[c])
        of_buf[b, rows, :] = stage_pv(rows, v_buf(b), b)

    def last_s(c):
        rows = pl.ds(*CH[c])
        stage_s(q_buf[rows, :], k_buf(0), rows)

    def last_o(c):
        rows = pl.ds(*CH[c])
        o2 = jnp.concatenate([normalize(of_buf[b, rows, :], rows, b) for b in range(2)], axis=1)
        wo2 = jnp.concatenate([wo_buf[0], wo_buf[1]], axis=0)
        acc[rows, :] = acc[rows, :] + _mm(o2, wo2)

    def last_fin(c):
        for r0 in range(CH[c][0], sum(CH[c]), 128):
            parts = []
            for g in range(r0, r0 + 128, RG):
                rows = slice(g, g + RG)
                x1 = x_buf[rows, :].astype(F32) + fin(0) * acc[rows, :]
                d = x1 - jnp.mean(x1, axis=-1, keepdims=True)
                rstd = jax.lax.rsqrt(jnp.mean(d * d, axis=-1, keepdims=True) + EPS)
                da = d * fin(1)
                part = da[:, 0:128]
                for j in range(1, KD):
                    part = part + da[:, j * 128:(j + 1) * 128]
                parts.append(part * rstd)
                o_stage[rows, :] = ((x1 + fin(3)) + (d * rstd) * fin(2)).astype(BF)
            blk = jnp.concatenate(parts, axis=0)
            r_buf[r0 // 128:r0 // 128 + 1, :] = jnp.sum(blk.T, axis=0, keepdims=True)
        out_copy(c).start()

    stages = (lambda c: last_pv(c, 0), last_s, lambda c: last_pv(c, 1), last_o, last_fin)
    for step in range(1, NC + len(stages) - 2):
        @pl.when(flag[0] == 1)
        def _():
            if step == 1:
                fin_consts()
            for lag in (2, 3, 0, 1, 4):
                if 0 <= step - lag < NC:
                    stages[lag](step - lag)
            if step == NC + 2:
                last_fin(NC - 1)

    ga, cb1, sb, gb = fin(0), fin(4), fin(5), fin(6)
    rr = r_buf[...] + jnp.sum(sb * fin(7), axis=-1, keepdims=True)
    row = (jax.lax.broadcasted_iota(jnp.int32, rr.shape, 0) * 128
           + jax.lax.broadcasted_iota(jnp.int32, rr.shape, 1))

    def top1(v):
        m = jnp.max(jnp.max(v, axis=0, keepdims=True), axis=1, keepdims=True)
        i = jnp.min(jnp.min(jnp.where(v == m, row, S - 1), axis=0, keepdims=True), axis=1, keepdims=True)
        return m, i

    m1v, i1v = top1(rr)
    m2v, i2v = top1(jnp.where(row == i1v, -jnp.inf, rr))
    i1, i2 = i1v[0, 0], i2v[0, 0]

    b1 = pl.multiple_of((i1 // 16) * 16, 16)
    b2 = pl.multiple_of((i2 // 16) * 16, 16)
    xs = (jnp.concatenate([x_buf[pl.ds(b1, 16), :], x_buf[pl.ds(b2, 16), :]], axis=0).astype(F32)
          + ga * jnp.concatenate([acc[pl.ds(b1, 16), :], acc[pl.ds(b2, 16), :]], axis=0))
    h2 = _ln_mod(xs, cb1, sb).astype(BF)
    h2f = h2.astype(F32)

    for t, buf in enumerate((wg_buf, wu_buf, wd_buf)):
        pltpu.make_async_copy(buf, buf, sem_moe.at[t]).wait()
    acts = []
    for j in range(FB):
        g = _mm(h2, wg_buf[j])
        u = _mm(h2, wu_buf[j])
        acts.append((g * jax.nn.sigmoid(g) * u).astype(BF))
    ys = []
    for n in range(KD):
        y = None
        for j in range(FB):
            t = _mm(acts[j], wd_buf[n, j * 128:(j + 1) * 128, :])
            y = t if y is None else y + t
        ys.append(y)
    y = jnp.concatenate(ys, axis=1)
    g1 = jax.nn.sigmoid(m1v)
    g2 = jax.nn.sigmoid(m2v)
    row16 = jax.lax.broadcasted_iota(jnp.int32, (16, D), 0)

    for i in range(NC):
        out_copy(i).wait()

    ya = y[0:16] * g1
    yb = y[16:32] * g2
    u1 = jnp.where(row16 == i1 - b1, ya, jnp.where(row16 == i2 - b1, yb, 0.0))
    u2 = jnp.where(row16 == i2 - b2, yb, jnp.where(row16 == i1 - b2, ya, 0.0))
    o_stage[pl.ds(b1, 16), :] = (xs[0:16] + gb * (h2f[0:16] + u1)).astype(BF)
    o_stage[pl.ds(b2, 16), :] = (xs[16:32] + gb * (h2f[16:32] + u2)).astype(BF)

    f1 = pltpu.make_async_copy(o_stage.at[pl.ds(b1, 16), :], out_hbm.at[pl.ds(b1, 16), :], sem_fix.at[0])
    f2 = pltpu.make_async_copy(o_stage.at[pl.ds(b2, 16), :], out_hbm.at[pl.ds(b2, 16), :], sem_fix.at[1])
    f1.start()

    @pl.when(b1 != b2)
    def _():
        f2.start()
        f2.wait()

    f1.wait()


@jax.jit
def pallas_adaLN_cond__mha_block_cached__moe_arch_mod__prompt_kernel(
    A_x: jax.Array,
    A_k_cache: jax.Array,
    A_v_cache: jax.Array,
    A_wq: jax.Array,
    A_wo: jax.Array,
    B_x: jax.Array,
    B_w_r: jax.Array,
    B_w_gate: jax.Array,
    B_w_up: jax.Array,
    B_w_down: jax.Array,
    c: jax.Array,
    w_mod: jax.Array,
):
    any_spec = pl.BlockSpec(memory_space=pl.ANY)
    out = pl.pallas_call(
        _kernel,
        out_shape=jax.ShapeDtypeStruct((S, D), BF),
        in_specs=[any_spec] * 11,
        out_specs=any_spec,
        scratch_shapes=[
            pltpu.VMEM((S, D), BF),
            pltpu.VMEM((S, D), BF),
            pltpu.VMEM((KD, S, 128), BF),
            pltpu.VMEM((S, D), F32),
            pltpu.VMEM((S, S), F32),
            pltpu.VMEM((S, 128), F32),
            pltpu.VMEM((2, S, 128), F32),
            pltpu.VMEM((2, NKB, S, 128), F32),
            pltpu.VMEM((S, DH), BF),
            pltpu.VMEM((2, 2 * S + 2 * D, 128), BF),
            pltpu.VMEM((2, DH, D), BF),
            pltpu.VMEM((D, DH), BF),
            pltpu.VMEM((2, D, D), BF),
            pltpu.VMEM((FB, D, 128), BF),
            pltpu.VMEM((FB, D, 128), BF),
            pltpu.VMEM((KD, F, 128), BF),
            pltpu.VMEM((1, D), BF),
            pltpu.VMEM((D,), BF),
            pltpu.VMEM((D, 128), F32),
            pltpu.VMEM((D, 128), F32),
            pltpu.VMEM((H, 8, 128), F32),
            pltpu.VMEM((8, 8, D), F32),
            pltpu.VMEM((S // 128, 128), F32),
            pltpu.SMEM((1,), jnp.int32),
            pltpu.SemaphoreType.DMA((2,)),
            pltpu.SemaphoreType.DMA((2,)),
            pltpu.SemaphoreType.DMA((NX,)),
            pltpu.SemaphoreType.DMA((2, M1C)),
            pltpu.SemaphoreType.DMA((3,)),
            pltpu.SemaphoreType.DMA((3,)),
            pltpu.SemaphoreType.DMA((NC,)),
            pltpu.SemaphoreType.DMA((2,)),
            pltpu.SemaphoreType.REGULAR,
        ],
        compiler_params=pltpu.CompilerParams(vmem_limit_bytes=120 << 20, disable_bounds_checks=True),
    )(
        A_x.reshape(S, D),
        A_k_cache.reshape(H, S, DH),
        A_v_cache.reshape(H, S, DH),
        A_wq,
        A_wo,
        B_w_r,
        B_w_gate,
        B_w_up,
        B_w_down,
        c,
        w_mod,
    )
    return out.reshape(1, S, D)
```

```python
import jax
import jax.numpy as jnp
import jax.experimental.pallas as pl
import jax.experimental.pallas.tpu as pltpu

S = 2048
D = 1024
H = 32
DH = 128
F = 3584
KB = 512
NKB = S // KB
RX = 512
NX = S // RX
RG = 16
CH = ((0, 512), (512, 512), (1024, 512), (1536, 256), (1792, 256))
NC = len(CH)
KD = D // 128
FB = F // 128
M1C = 4
MR = D // M1C
EPS = 1e-5
LOG2E = 1.4426950408889634
QSCALE = (DH ** -0.5) * LOG2E
BF = jnp.bfloat16
F32 = jnp.float32


def _ln_mod(xf, mul, add):
    mu = jnp.mean(xf, axis=-1, keepdims=True)
    d = xf - mu
    var = jnp.mean(d * d, axis=-1, keepdims=True)
    return d * jax.lax.rsqrt(var + EPS) * mul + add


def _mm(a, b):
    return jnp.dot(a, b, preferred_element_type=F32)


def _kernel(x_hbm, k_hbm, v_hbm, wq_hbm, wo_hbm, wr_hbm, wg_hbm, wu_hbm, wd_hbm,
            c_hbm, wm_hbm, out_hbm,
            x_buf, o_stage, h_buf, acc, s_buf, m_buf, of_buf, l_buf,
            q_buf, pk_buf, wo_buf, wq0_buf,
            wm1_buf, wg_buf, wu_buf, wd_buf, c_buf, wr_buf, scol, sa_col, mod_buf, fin_buf, r_buf, flag,
            sem_pk, sem_wo, sem_x, sem_m1, sem_small, sem_moe, sem_out, sem_fix, sem_fence):
    def k_buf(slot):
        return pk_buf.at[slot, pl.ds(0, S), :]

    def wq_buf(slot):
        return pk_buf.at[slot, pl.ds(S, D), :]

    def v_buf(slot):
        return pk_buf.at[slot, pl.ds(S + D, S), :]

    def wm_buf(slot):
        return pk_buf.at[slot, pl.ds(2 * S + D, D), :]

    def cp_k(h, slot):
        return pltpu.make_async_copy(k_hbm.at[h], k_buf(slot), sem_pk.at[slot])

    def cp_v(h, slot):
        return pltpu.make_async_copy(v_hbm.at[h], v_buf(slot), sem_pk.at[slot])

    def cp_wq(h, slot):
        return pltpu.make_async_copy(wq_hbm.at[:, pl.ds(h * DH, DH)], wq_buf(slot), sem_pk.at[slot])

    def cp_wm(h, slot):
        return pltpu.make_async_copy(wm_hbm.at[:, pl.ds(2 * D + h * 128, 128)], wm_buf(slot), sem_pk.at[slot])

    def cp_wo(h, slot):
        return pltpu.make_async_copy(wo_hbm.at[pl.ds(h * DH, DH), :], wo_buf.at[slot], sem_wo.at[slot])

    def wait_packet(slot, last=False):
        dst = pk_buf.at[slot, pl.ds(S + D, S + D), :] if last else pk_buf.at[slot]
        pltpu.make_async_copy(dst, dst, sem_pk.at[slot]).wait()
        cp_wo(0, slot).wait()

    def packet(h, slot, last=False):
        cps = [] if last else [cp_wq(h + 1, slot)]
        cps += [cp_v(h, slot), cp_wm(h, slot)]
        if not last:
            cps.append(cp_k(h + 1, slot))
        cps.append(cp_wo(h, slot))
        return cps

    def x_copy(i):
        rows = pl.ds(i * RX, RX)
        return pltpu.make_async_copy(x_hbm.at[rows, :], x_buf.at[rows, :], sem_x.at[i])

    def m1_copy(k, i):
        return pltpu.make_async_copy(wm_hbm.at[pl.ds(i * MR, MR), pl.ds(k * D, D)],
                                     wm1_buf.at[k, pl.ds(i * MR, MR), :], sem_m1.at[k, i])

    def moe_copies(j):
        return [
            pltpu.make_async_copy(wg_hbm.at[:, pl.ds(j * 128, 128)], wg_buf.at[j], sem_moe.at[0]),
            pltpu.make_async_copy(wu_hbm.at[:, pl.ds(j * 128, 128)], wu_buf.at[j], sem_moe.at[1]),
        ]

    def wd_copy(n):
        return pltpu.make_async_copy(wd_hbm.at[:, pl.ds(n * 128, 128)], wd_buf.at[n], sem_moe.at[2])

    def out_copy(i):
        rows = pl.ds(*CH[i])
        return pltpu.make_async_copy(o_stage.at[rows, :], out_hbm.at[rows, :], sem_out.at[i])

    c_copy = pltpu.make_async_copy(c_hbm, c_buf, sem_small.at[0])
    wr_copy = pltpu.make_async_copy(wr_hbm, wr_buf, sem_small.at[1])
    wq0_copy = pltpu.make_async_copy(wq_hbm.at[:, pl.ds(0, DH)], wq0_buf, sem_small.at[2])

    def start_in_order(*cps):
        for cp in cps:
            cp.start()
            pl.semaphore_signal(sem_fence, 1)
            pl.semaphore_wait(sem_fence, 1)

    def q_bias(wq):
        return jnp.sum(wq[...].astype(F32) * sa_col[...], axis=0, keepdims=True)

    def stage_q(wq):
        q = None
        for j in range(KD):
            t = _mm(h_buf[j], wq[j * 128:(j + 1) * 128, :])
            q = t if q is None else q + t
        return ((q + q_bias(wq)) * QSCALE).astype(BF)

    def qk_round(q, t, k_ref, rows, mx):
        s = jax.lax.dot_general(q, k_ref[t * KB:(t + 1) * KB, :], (((1,), (1,)), ((), ())),
                                preferred_element_type=F32)
        s_buf[rows, t * KB:(t + 1) * KB] = s
        for j in range(KB // 128):
            sj = s[:, j * 128:(j + 1) * 128]
            mx = sj if mx is None else jnp.maximum(mx, sj)
        return mx

    def row_max(mx):
        return jnp.broadcast_to(jnp.max(mx, axis=-1, keepdims=True), mx.shape)

    def stage_s(q, k_ref, rows=slice(None)):
        mx = None
        for t in range(NKB):
            mx = qk_round(q, t, k_ref, rows, mx)
        m_buf[rows, :] = row_max(mx)

    def stage_pv(rows, v_ref, b=0):
        m = m_buf[rows, :]
        m = jnp.concatenate([m] * (KB // 128), axis=1)
        o = None
        for t in range(NKB):
            p = jnp.exp2(s_buf[rows, t * KB:(t + 1) * KB] - m)
            l = p[:, 0:128]
            for j in range(1, KB // 128):
                l = l + p[:, j * 128:(j + 1) * 128]
            l_buf[b, t, rows, :] = l
            ot = _mm(p.astype(BF), v_ref[t * KB:(t + 1) * KB, :])
            o = ot if o is None else o + ot
        return o

    def normalize(o, rows, b=0):
        l = l_buf[b, 0, rows, :]
        for t in range(1, NKB):
            l = l + l_buf[b, t, rows, :]
        l = jnp.sum(l, axis=-1, keepdims=True)
        return (o * pltpu.reciprocal(l, full_range=False)).astype(BF)

    def stage_mod(h, slot):
        w = wm_buf(slot)[...].astype(F32) * scol[...]
        mod_buf[h] = jnp.broadcast_to(jnp.sum(w, axis=0, keepdims=True), (8, 128))

    def head_step(h, slot):
        allr = slice(None)
        stage_mod(h, slot)
        q_buf[...] = stage_q(wq_buf(slot))
        o = stage_pv(allr, v_buf(slot))
        stage_s(q_buf[...], k_buf(slot))
        acc[...] = jnp.where(h > 0, acc[...], 0.0) + _mm(normalize(o, allr), wo_buf[slot])

    flag[0] = 1
    start_in_order(c_copy, *[x_copy(i) for i in range(NX)], wq0_copy, *[m1_copy(1, i) for i in range(M1C)],
                   *[m1_copy(0, i) for i in range(M1C)], cp_k(0, 1))

    c_copy.wait()
    cf = c_buf[...].astype(F32)
    sc = (cf * jax.nn.sigmoid(cf)).astype(BF)
    sc16 = jnp.broadcast_to(sc, (16, D))
    scf = sc.astype(F32)
    for j in range(KD):
        blk = jnp.broadcast_to(scf[:, j * 128:(j + 1) * 128], (128, 128))
        scol[j * 128:(j + 1) * 128, :] = blk.T

    for i in range(NX):
        x_copy(i).wait()
        for g in range(i * RX, (i + 1) * RX, RG):
            xf = x_buf[g:g + RG, :].astype(F32)
            mu = jnp.mean(xf, axis=-1, keepdims=True)
            d = xf - mu
            acc[g:g + RG, :] = d * jax.lax.rsqrt(jnp.mean(d * d, axis=-1, keepdims=True) + EPS)

    def mod1(k):
        m = None
        for i in range(M1C):
            if k == 1:
                m1_copy(k, i).wait()
            elif i == 0:
                for ii in range(M1C):
                    m1_copy(k, ii).wait()
            t = _mm(sc16[:, i * MR:(i + 1) * MR], wm1_buf[k, i * MR:(i + 1) * MR, :])
            m = t if m is None else m + t
        return m[0:1, :].astype(BF).astype(F32)

    ca1 = (1.0 + mod1(1)).astype(BF).astype(F32)
    for cp in packet(0, 0):
        cp.start()
    wr_copy.start()
    wq0_copy.wait()
    q0 = None
    for j in range(KD):
        cols = slice(j * 128, (j + 1) * 128)
        hj = (acc[:, cols] * ca1[:, cols]).astype(BF)
        h_buf[j] = hj
        t = _mm(hj, wq0_buf[cols, :])
        q0 = t if q0 is None else q0 + t
    of_buf[0] = q0
    sa = mod1(0)
    cp_k(0, 1).wait()
    for j in range(KD):
        sa_col[j * 128:(j + 1) * 128, :] = jnp.broadcast_to(sa[:, j * 128:(j + 1) * 128], (128, 128)).T
    bias = _mm(jnp.broadcast_to(sa, (16, D)).astype(BF), wq0_buf[...])[0:1, :]
    q_buf[...] = ((of_buf[0] + bias) * QSCALE).astype(BF)
    stage_s(q_buf[...], k_buf(1))

    def loop(h, carry):
        slot = h & 1
        wait_packet(slot)

        @pl.when(h < FB)
        def _():
            for cp in moe_copies(h):
                cp.start()

        @pl.when(h < KD)
        def _():
            wd_copy(h).start()

        cp_wq(h + 2, 1 - slot).start()
        cp_k(h + 2, 1 - slot).start()
        cp_v(h + 1, 1 - slot).start()
        cp_wm(h + 1, 1 - slot).start()
        cp_wo(h + 1, 1 - slot).start()
        head_step(h, slot)
        return carry

    jax.lax.fori_loop(0, H - 2, loop, 0)

    for cp in packet(H - 1, 1, last=True):
        cp.start()
    wait_packet(0)
    wr_copy.wait()
    stage_mod(H - 2, 0)
    q_buf[...] = stage_q(wq_buf(0))
    rows0 = pl.ds(*CH[0])
    of_buf[0, rows0, :] = stage_pv(rows0, v_buf(0))
    wait_packet(1, last=True)

    def mod_row(i):
        return jnp.concatenate([mod_buf[i * KD + j][0:1, :] for j in range(KD)], axis=1).astype(BF).astype(F32)

    def fin_consts():
        stage_mod(H - 1, 1)
        cb1 = (1.0 + mod_row(2)).astype(BF).astype(F32)
        sb, gb = mod_row(1), mod_row(3)
        wr = wr_buf[...].astype(F32).reshape(1, D)
        for i, row in enumerate([mod_row(0), cb1 * wr, gb * cb1, gb * sb, cb1, sb, gb, wr]):
            fin_buf[i] = jnp.broadcast_to(row, (8, D))

    def fin(i):
        return fin_buf[i][0:1, :]

    def last_pv(c, b):
        rows = pl.ds(*CH[c])
        of_buf[b, rows, :] = stage_pv(rows, v_buf(b), b)

    def last_s(c):
        rows = pl.ds(*CH[c])
        stage_s(q_buf[rows, :], k_buf(0), rows)

    def last_o(c):
        rows = pl.ds(*CH[c])
        o2 = jnp.concatenate([normalize(of_buf[b, rows, :], rows, b) for b in range(2)], axis=1)
        wo2 = jnp.concatenate([wo_buf[0], wo_buf[1]], axis=0)
        acc[rows, :] = acc[rows, :] + _mm(o2, wo2)

    def last_fin(c):
        for r0 in range(CH[c][0], sum(CH[c]), 128):
            parts = []
            for g in range(r0, r0 + 128, 32):
                rows = slice(g, g + 32)
                x1 = x_buf[rows, :].astype(F32) + fin(0) * acc[rows, :]
                d = x1 - jnp.mean(x1, axis=-1, keepdims=True)
                rstd = jax.lax.rsqrt(jnp.mean(d * d, axis=-1, keepdims=True) + EPS)
                u = d * rstd
                da = u * fin(1)
                part = da[:, 0:128]
                for j in range(1, KD):
                    part = part + da[:, j * 128:(j + 1) * 128]
                parts.append(part)
                o_stage[rows, :] = ((x1 + fin(3)) + u * fin(2)).astype(BF)
            blk = jnp.concatenate(parts, axis=0)
            r_buf[r0 // 128:r0 // 128 + 1, :] = jnp.sum(blk.T, axis=0, keepdims=True)
        out_copy(c).start()

    stages = (lambda c: last_pv(c, 0), last_s, lambda c: last_pv(c, 1), last_o, last_fin)
    for step in range(1, NC + len(stages) - 2):
        @pl.when(flag[0] == 1)
        def _():
            if step == 1:
                fin_consts()
            for lag in (4, 2, 0, 3, 1):
                if 0 <= step - lag < NC:
                    stages[lag](step - lag)
            if step == NC + 2:
                last_fin(NC - 1)

    ga, cb1, sb, gb = fin(0), fin(4), fin(5), fin(6)
    rr = r_buf[...] + jnp.sum(sb * fin(7), axis=-1, keepdims=True)
    row = (jax.lax.broadcasted_iota(jnp.int32, rr.shape, 0) * 128
           + jax.lax.broadcasted_iota(jnp.int32, rr.shape, 1))

    def top1(v):
        m = jnp.max(jnp.max(v, axis=0, keepdims=True), axis=1, keepdims=True)
        i = jnp.min(jnp.min(jnp.where(v == m, row, S - 1), axis=0, keepdims=True), axis=1, keepdims=True)
        return m, i

    m1v, i1v = top1(rr)
    m2v, i2v = top1(jnp.where(row == i1v, -jnp.inf, rr))
    i1, i2 = i1v[0, 0], i2v[0, 0]

    b1 = pl.multiple_of((i1 // 16) * 16, 16)
    b2 = pl.multiple_of((i2 // 16) * 16, 16)
    xs = (jnp.concatenate([x_buf[pl.ds(b1, 16), :], x_buf[pl.ds(b2, 16), :]], axis=0).astype(F32)
          + ga * jnp.concatenate([acc[pl.ds(b1, 16), :], acc[pl.ds(b2, 16), :]], axis=0))
    h2 = _ln_mod(xs, cb1, sb).astype(BF)
    h2f = h2.astype(F32)

    for t, buf in enumerate((wg_buf, wu_buf, wd_buf)):
        pltpu.make_async_copy(buf, buf, sem_moe.at[t]).wait()
    acts = []
    for j in range(FB):
        g = _mm(h2, wg_buf[j])
        u = _mm(h2, wu_buf[j])
        acts.append((g * jax.nn.sigmoid(g) * u).astype(BF))
    ys = []
    for n in range(KD):
        y = None
        for j in range(FB):
            t = _mm(acts[j], wd_buf[n, j * 128:(j + 1) * 128, :])
            y = t if y is None else y + t
        ys.append(y)
    y = jnp.concatenate(ys, axis=1)
    g1 = jax.nn.sigmoid(m1v)
    g2 = jax.nn.sigmoid(m2v)
    row16 = jax.lax.broadcasted_iota(jnp.int32, (16, D), 0)

    for i in range(NC):
        out_copy(i).wait()

    ya = y[0:16] * g1
    yb = y[16:32] * g2
    u1 = jnp.where(row16 == i1 - b1, ya, jnp.where(row16 == i2 - b1, yb, 0.0))
    u2 = jnp.where(row16 == i2 - b2, yb, jnp.where(row16 == i1 - b2, ya, 0.0))
    o_stage[pl.ds(b1, 16), :] = (xs[0:16] + gb * (h2f[0:16] + u1)).astype(BF)
    o_stage[pl.ds(b2, 16), :] = (xs[16:32] + gb * (h2f[16:32] + u2)).astype(BF)

    f1 = pltpu.make_async_copy(o_stage.at[pl.ds(b1, 16), :], out_hbm.at[pl.ds(b1, 16), :], sem_fix.at[0])
    f2 = pltpu.make_async_copy(o_stage.at[pl.ds(b2, 16), :], out_hbm.at[pl.ds(b2, 16), :], sem_fix.at[1])
    f1.start()

    @pl.when(b1 != b2)
    def _():
        f2.start()
        f2.wait()

    f1.wait()


@jax.jit
def pallas_adaLN_cond__mha_block_cached__moe_arch_mod__prompt_kernel(
    A_x: jax.Array,
    A_k_cache: jax.Array,
    A_v_cache: jax.Array,
    A_wq: jax.Array,
    A_wo: jax.Array,
    B_x: jax.Array,
    B_w_r: jax.Array,
    B_w_gate: jax.Array,
    B_w_up: jax.Array,
    B_w_down: jax.Array,
    c: jax.Array,
    w_mod: jax.Array,
):
    any_spec = pl.BlockSpec(memory_space=pl.ANY)
    out = pl.pallas_call(
        _kernel,
        out_shape=jax.ShapeDtypeStruct((S, D), BF),
        in_specs=[any_spec] * 11,
        out_specs=any_spec,
        scratch_shapes=[
            pltpu.VMEM((S, D), BF),
            pltpu.VMEM((S, D), BF),
            pltpu.VMEM((KD, S, 128), BF),
            pltpu.VMEM((S, D), F32),
            pltpu.VMEM((S, S), F32),
            pltpu.VMEM((S, 128), F32),
            pltpu.VMEM((2, S, 128), F32),
            pltpu.VMEM((2, NKB, S, 128), F32),
            pltpu.VMEM((S, DH), BF),
            pltpu.VMEM((2, 2 * S + 2 * D, 128), BF),
            pltpu.VMEM((2, DH, D), BF),
            pltpu.VMEM((D, DH), BF),
            pltpu.VMEM((2, D, D), BF),
            pltpu.VMEM((FB, D, 128), BF),
            pltpu.VMEM((FB, D, 128), BF),
            pltpu.VMEM((KD, F, 128), BF),
            pltpu.VMEM((1, D), BF),
            pltpu.VMEM((D,), BF),
            pltpu.VMEM((D, 128), F32),
            pltpu.VMEM((D, 128), F32),
            pltpu.VMEM((H, 8, 128), F32),
            pltpu.VMEM((8, 8, D), F32),
            pltpu.VMEM((S // 128, 128), F32),
            pltpu.SMEM((1,), jnp.int32),
            pltpu.SemaphoreType.DMA((2,)),
            pltpu.SemaphoreType.DMA((2,)),
            pltpu.SemaphoreType.DMA((NX,)),
            pltpu.SemaphoreType.DMA((2, M1C)),
            pltpu.SemaphoreType.DMA((3,)),
            pltpu.SemaphoreType.DMA((3,)),
            pltpu.SemaphoreType.DMA((NC,)),
            pltpu.SemaphoreType.DMA((2,)),
            pltpu.SemaphoreType.REGULAR,
        ],
        compiler_params=pltpu.CompilerParams(vmem_limit_bytes=120 << 20, disable_bounds_checks=True),
    )(
        A_x.reshape(S, D),
        A_k_cache.reshape(H, S, DH),
        A_v_cache.reshape(H, S, DH),
        A_wq,
        A_wo,
        B_w_r,
        B_w_gate,
        B_w_up,
        B_w_down,
        c,
        w_mod,
    )
    return out.reshape(1, S, D)
```
